```python
import jax
import jax.numpy as jnp

def _softmax(x, axis=-1):
    return jax.nn.softmax(x, axis=axis)
def _gelu(x):
    return jax.nn.gelu(x, approximate=True)
def _silu(x):
    return jax.nn.silu(x)
def _sigmoid(x):
    return jax.nn.sigmoid(x)
def _layernorm(x, axis=-1, eps=1e-5):
    m = jnp.mean(x, axis=axis, keepdims=True)
    v = jnp.var(x, axis=axis, keepdims=True)
    return (x - m) / jnp.sqrt(v + eps)
def _scatter_add(tgt, idx, src, axis=0):
    return tgt.at[idx].add(src)
def _segment_sum(src, seg, n):
    return jax.ops.segment_sum(src, seg, n)
class _Rng:
    def __init__(self, key):
        self._k = key
    def _next(self):
        self._k, sub = jax.random.split(self._k)
        return sub
    def normal(self, shape):
        return jax.random.normal(self._next(), shape, dtype=jnp.bfloat16)
    def randint(self, lo, hi, shape):
        return jax.random.randint(self._next(), shape, lo, hi, dtype=jnp.int32)
    def uniform(self, shape, lo=0.0, hi=1.0):
        return jax.random.uniform(self._next(), shape, jnp.bfloat16, lo, hi)
    def permutation(self, n):
        return jax.random.permutation(self._next(), n)


kernel_name = 'parallel_sum__sliding_local_dilated__glu_gated_bilinear__prompt'

def setup_inputs():
    _rng = _Rng(jax.random.key(int.from_bytes(__import__("os").urandom(4), "little")))
    _w = (lambda a: (lambda t: t.astype(jnp.bfloat16) if jnp.issubdtype(t.dtype, jnp.floating) else t)(jnp.asarray(a)))
    def _A_setup():
        B, S, D = 1, 2048, 1024
        return {
            "x": _w((lambda *s: _rng.normal(s) * 0.05)(B, S, D)),
            "wqkv": _w((lambda *s: _rng.normal(s) * 0.05)(D, 3 * D)),
            "wo": _w((lambda *s: _rng.normal(s) * 0.05)(D, D)),
        }
    _A_in = _A_setup()

    def _B_setup():
        B, S, D, F = 1, 2048, 1024, 3584
        return {
            "x": _w((lambda *s: _rng.normal(s) * 0.05)(B, S, D)),
            "w_gate": _w((lambda *s: _rng.normal(s) * 0.05)(D, F) * (D ** -0.5)),
            "w_up": _w((lambda *s: _rng.normal(s) * 0.05)(D, F) * (D ** -0.5)),
            "w_down": _w((lambda *s: _rng.normal(s) * 0.05)(F, D) * (F ** -0.5)),
        }
    _B_in = _B_setup()

    return {
        "A_x": _A_in["x"],
        "A_wqkv": _A_in["wqkv"],
        "A_wo": _A_in["wo"],
        "B_x": _B_in["x"],
        "B_w_gate": _B_in["w_gate"],
        "B_w_up": _B_in["w_up"],
        "B_w_down": _B_in["w_down"],
    }

def reference(A_x, A_wqkv, A_wo, B_x, B_w_gate, B_w_up, B_w_down):
    def _A_ref(x, wqkv, wo):
        B, S, D = x.shape
        H = 32; Dh = D // H
        W, dil = 8, 2
        qkv = (lambda x, *d: x.transpose(*d))((x @ wqkv).reshape(B, S, 3, H, Dh), 2, 0, 3, 1, 4)
        q, k, v = qkv[0], qkv[1], qkv[2]
        scale = Dh ** -0.5
        pos = jnp.arange(S)
        off = jnp.arange(W) * dil
        idx = pos[:, None] - off[None, :]
        mask = idx >= 0
        idx_c = jnp.where(mask, idx, 0).reshape(-1)
        kg = k[:, :, idx_c, :].reshape(B, H, S, W, Dh)
        vg = v[:, :, idx_c, :].reshape(B, H, S, W, Dh)
        logits = jnp.einsum("bhsd,bhswd->bhsw", q, kg) * scale
        logits = jnp.where(mask[None, None, :, :], logits, -1e9)
        attn = _softmax(logits, axis=-1)
        o = jnp.einsum("bhsw,bhswd->bhsd", attn, vg)
        return (lambda x, *d: x.transpose(*d))(o, 0, 2, 1, 3).reshape(B, S, D) @ wo

    def _B_ref(x, w_gate, w_up, w_down):
        g = jnp.einsum("bsd,df->bsf", x, w_gate)
        u = jnp.einsum("bsd,df->bsf", x, w_up)
        h = g * u
        return jnp.einsum("bsf,fd->bsd", h, w_down)

    x = A_x
    xn = _layernorm(x, axis=-1)
    return x + _A_ref(xn, A_wqkv, A_wo) + _B_ref(xn, B_w_gate, B_w_up, B_w_down)
```

```python
import functools

import jax
import jax.numpy as jnp
import jax.experimental.pallas as pl
import jax.experimental.pallas.tpu as pltpu

F32, BF16 = jnp.float32, jnp.bfloat16
HEAD_DIM, WINDOW, DILATION, EPS = 32, 8, 2, 1e-5
LANES, PAD = 128, 16


def _dot(a, b):
    return jnp.dot(a, b, preferred_element_type=F32)


def _lhs7(a11, a12, a21, a22):
    return [a11 + a22, a21 + a22, a11, a22, a11 + a12, a21 - a11, a12 - a22]


def _rhs7(b11, b12, b21, b22):
    return [b11 + b22, b11, b12 - b22, b21 - b11, b22, b11 + b12, b21 + b22]


def _out4(m):
    return (m[0] + m[3] - m[4] + m[6], m[2] + m[4], m[1] + m[3], m[0] - m[1] + m[2] + m[5])


def _outer(fn, blk):
    return [[fn(blk[i][j], blk[i][j + 2], blk[i + 2][j], blk[i + 2][j + 2]) for j in range(2)] for i in range(2)]


def _inner(fn, outer):
    res = []
    for o in range(7):
        res += fn(outer[0][0][o], outer[0][1][o], outer[1][0][o], outer[1][1][o])
    return res


def _out16(m):
    inner = [_out4(m[7 * o:7 * o + 7]) for o in range(7)]
    out = [[None] * 4 for _ in range(4)]
    for i in range(2):
        for j in range(2):
            c = _out4([inner[o][2 * i + j] for o in range(7)])
            out[i][j], out[i][j + 2], out[i + 2][j], out[i + 2][j + 2] = c
    return out


def _swap_block_lane(blocks):
    lane = jax.lax.broadcasted_iota(jnp.int32, blocks[0].shape, 1)
    t = [x if b == 0 else pltpu.roll(x, b, 1) for b, x in enumerate(blocks)]
    s = [t[(-c) % 8] for c in range(8)]
    for bit in (1, 2, 4):
        m = (lane & bit) != 0
        s = [jnp.where(m, s[(c - bit) % 8], s[c]) for c in range(8)]
    return [x if c == 0 else pltpu.roll(x, LANES - c, 1) for c, x in enumerate(s)]


def _attention(qkv_s, row, n):
    lane = jax.lax.broadcasted_iota(jnp.int32, (n, LANES), 1)
    pos = jax.lax.broadcasted_iota(jnp.int32, (n, LANES), 0) + row
    q = [qkv_s[0, c, pl.ds(row + PAD, n), :] for c in range(8)]
    logits = []
    for w in range(WINDOW):
        rows = pl.ds(row + (PAD - DILATION * w), n)
        s = q[0] * qkv_s[1, 0, rows, :]
        for c in range(1, 8):
            s = s + q[c] * qkv_s[1, c, rows, :]
        s = s + pltpu.roll(s, LANES - 8, 1)
        s = s + pltpu.roll(s, LANES - 16, 1)
        s = s * (HEAD_DIM ** -0.5)
        if w:
            s = jnp.where(pos >= DILATION * w, s, -1e9)
        logits.append(s)
    m = functools.reduce(jnp.maximum, logits)
    e = [jnp.exp(s - m) for s in logits]
    inv = 1.0 / functools.reduce(lambda a, b: a + b, e)
    p = []
    for w in range(WINDOW):
        a = e[w] * inv
        a = jnp.where((lane & 24) == 0, a, pltpu.roll(a, 8, 1))
        a = jnp.where((lane & 16) == 0, a, pltpu.roll(a, 16, 1))
        p.append(a)
    out = []
    for c in range(8):
        o = p[0] * qkv_s[2, c, pl.ds(row + PAD, n), :]
        for w in range(1, WINDOW):
            o = o + p[w] * qkv_s[2, c, pl.ds(row + (PAD - DILATION * w), n), :]
        out.append(o)
    return _swap_block_lane(out)


def _kernel(x_hbm, wqkv_hbm, wo_hbm, wg_hbm, wu_hbm, wd_hbm, out_hbm,
            x_v, wqkv_v, wo_v, wg_v, wu_v, wd_v, a1, a2, acc, qkv_s,
            x_sem, w_sem, f_sem, o_sem, *, tf, nxg, nog):
    _, qm, d = x_v.shape
    hm, hd, qd, qf = 2 * qm, d // 2, d // 4, tf // 4
    nf = wg_hbm.shape[1] // tf
    xr = qm // nxg
    orows = qm // nog

    def x_copy(g):
        r = pl.ds(g * xr, xr)
        return pltpu.make_async_copy(x_hbm.at[:, r, :], x_v.at[:, r, :], x_sem.at[g])

    def w_copy(m):
        return pltpu.make_async_copy(wqkv_hbm.at[:, pl.ds(m * d, d)], wqkv_v.at[m], w_sem.at[m])

    wo_copy = pltpu.make_async_copy(wo_hbm, wo_v, w_sem.at[3])

    def f_copies(j, slot):
        c = pl.ds(pl.multiple_of(j * tf, tf), tf)
        return (pltpu.make_async_copy(wg_hbm.at[:, c], wg_v.at[slot], f_sem.at[0, slot]),
                pltpu.make_async_copy(wu_hbm.at[:, c], wu_v.at[slot], f_sem.at[1, slot]),
                pltpu.make_async_copy(wd_hbm.at[c, :], wd_v.at[slot], f_sem.at[2, slot]))

    def o_copy(g):
        r = pl.ds(pl.multiple_of(g * orows, orows), orows)
        return pltpu.make_async_copy(x_v.at[:, r, :], out_hbm.at[:, r, :], o_sem.at[g])

    for g in range(nxg):
        x_copy(g).start()
    for m in range(3):
        w_copy(m).start()
    for c in f_copies(0, 0):
        c.start()
    wo_copy.start()

    def ln_body(i, carry):
        r0 = pl.multiple_of(i * 16, 16)

        @pl.when(r0 % xr == 0)
        def _():
            x_copy(r0 // xr).wait()

        r = pl.ds(r0, 16)
        blk = []
        for q in range(4):
            x = x_v[q, r, :].astype(F32)
            xc = x - jnp.mean(x, axis=-1, keepdims=True)
            xn = xc * jax.lax.rsqrt(jnp.mean(xc * xc, axis=-1, keepdims=True) + EPS)
            blk.append([xn[:, p * qd:(p + 1) * qd] for p in range(4)])
        outer = _outer(_lhs7, blk)
        for o in range(7):
            for a in range(2):
                for b in range(2):
                    a1[o, pl.ds(a * qm + r0, 16), b * qd:(b + 1) * qd] = outer[a][b][o].astype(BF16)
        for t, v in enumerate(_inner(_lhs7, outer)):
            a2[t, r, :] = v.astype(BF16)
            acc[t, r, :] = jnp.zeros((16, qd), F32)
        return carry

    jax.lax.fori_loop(0, qm // 16, ln_body, 0)

    def qkv_body(m, carry):
        w_copy(m).wait()
        halves = []
        for i in range(2):
            blocks = [pltpu.bitcast(wqkv_v[m, i * hd:(i + 1) * hd, b * LANES:(b + 1) * LANES], jnp.uint32)
                      for b in range(8)]
            blocks = [pltpu.bitcast(x, BF16).astype(F32) for x in _swap_block_lane(blocks)]
            halves += [jnp.concatenate(blocks[:4], axis=1), jnp.concatenate(blocks[4:], axis=1)]
        rhs = _rhs7(*halves)
        c = _out4([_dot(a1[o], rhs[o].astype(BF16)) for o in range(7)])
        for a in range(2):
            for b in range(2):
                for p in range(4):
                    qkv_s[m, 4 * b + p, PAD + a * hm:PAD + (a + 1) * hm, :] = c[2 * a + b][:, p * LANES:(p + 1) * LANES]
        return carry

    jax.lax.fori_loop(0, 3, qkv_body, 0)
    for m in (1, 2):
        for c in range(8):
            qkv_s[m, c, :PAD, :] = jnp.broadcast_to(qkv_s[m, c, PAD:PAD + 1, :], (PAD, LANES))

    groups = -(-hm // (16 * nf))

    def w_blocks(ref, slot, r, c):
        return [[ref[slot, i * r:(i + 1) * r, j * c:(j + 1) * c].astype(F32) for j in range(4)] for i in range(4)]

    def ffn_body(j, carry):
        slot = j % 2

        @pl.when(j + 1 < nf)
        def _():
            for c in f_copies(j + 1, 1 - slot):
                c.start()

        for c in f_copies(j, slot):
            c.wait()
        bg = _inner(_rhs7, _outer(_rhs7, w_blocks(wg_v, slot, qd, qf)))
        bu = _inner(_rhs7, _outer(_rhs7, w_blocks(wu_v, slot, qd, qf)))
        bd = _inner(_rhs7, _outer(_rhs7, w_blocks(wd_v, slot, qf, qd)))
        g = _out16([_dot(a2[t], bg[t].astype(BF16)) for t in range(49)])
        u = _out16([_dot(a2[t], bu[t].astype(BF16)) for t in range(49)])
        h = [[g[a][b] * u[a][b] for b in range(4)] for a in range(4)]
        ha = _inner(_lhs7, _outer(_lhs7, h))
        for t in range(49):
            acc[t] += _dot(ha[t].astype(BF16), bd[t].astype(BF16))

        base = jnp.minimum(j * (16 * groups), hm - 16 * groups)
        for i in range(groups):
            r0 = pl.multiple_of(base + 16 * i, 16)
            top = _attention(qkv_s, r0, 16)
            bot = _attention(qkv_s, r0 + hm, 16)
            for p in range(4):
                for o, v in enumerate(_lhs7(top[p], top[p + 4], bot[p], bot[p + 4])):
                    a1[o, pl.ds(r0, 16), p * LANES:(p + 1) * LANES] = v.astype(BF16)
        return carry

    jax.lax.fori_loop(0, nf, ffn_body, 0)

    wo_copy.wait()

    def out_body(g, carry):
        r0 = pl.multiple_of(g * orows, orows)
        r = pl.ds(r0, orows)
        rhs = _rhs7(wo_v[:hd, :hd].astype(F32), wo_v[:hd, hd:].astype(F32),
                    wo_v[hd:, :hd].astype(F32), wo_v[hd:, hd:].astype(F32))
        m = []
        for o in range(7):
            lhs = jnp.concatenate([a1[o, r, :], a1[o, pl.ds(qm + r0, orows), :]], axis=0)
            p = _dot(lhs, rhs[o].astype(BF16))
            c = _out4([acc[7 * o + t, r, :] for t in range(7)])
            m.append([[p[a * orows:(a + 1) * orows, b * qd:(b + 1) * qd] + c[2 * a + b] for b in range(2)]
                      for a in range(2)])
        for a in range(2):
            for b in range(2):
                c = _out4([m[o][a][b] for o in range(7)])
                for i in range(2):
                    for k in range(2):
                        cols = slice((b + 2 * k) * qd, (b + 2 * k + 1) * qd)
                        x_v[a + 2 * i, r, cols] = (x_v[a + 2 * i, r, cols].astype(F32) + c[2 * i + k]).astype(BF16)
        o_copy(g).start()
        return carry

    jax.lax.fori_loop(0, nog, out_body, 0)
    for g in range(nog):
        o_copy(g).wait()


def make(tf=512, nxg=4, nog=4, flags=None):
    def fn(A_x, A_wqkv, A_wo, B_x, B_w_gate, B_w_up, B_w_down):
        del B_x
        b, s, d = A_x.shape
        qm = s // 4
        any_spec = pl.BlockSpec(memory_space=pl.ANY)
        out = pl.pallas_call(
            functools.partial(_kernel, tf=tf, nxg=nxg, nog=nog),
            in_specs=[any_spec] * 6,
            out_specs=any_spec,
            out_shape=jax.ShapeDtypeStruct((4, qm, d), A_x.dtype),
            scratch_shapes=[
                pltpu.VMEM((4, qm, d), BF16),
                pltpu.VMEM((3, d, d), BF16),
                pltpu.VMEM((d, d), BF16),
                pltpu.VMEM((2, d, tf), BF16),
                pltpu.VMEM((2, d, tf), BF16),
                pltpu.VMEM((2, tf, d), BF16),
                pltpu.VMEM((7, 2 * qm, d // 2), BF16),
                pltpu.VMEM((49, qm, d // 4), BF16),
                pltpu.VMEM((49, qm, d // 4), F32),
                pltpu.VMEM((3, 8, PAD + s, LANES), F32),
                pltpu.SemaphoreType.DMA((nxg,)),
                pltpu.SemaphoreType.DMA((4,)),
                pltpu.SemaphoreType.DMA((3, 2)),
                pltpu.SemaphoreType.DMA((nog,)),
            ],
            compiler_params=pltpu.CompilerParams(vmem_limit_bytes=125 * 2 ** 20, flags=flags),
        )(A_x.reshape(4, qm, d), A_wqkv, A_wo, B_w_gate, B_w_up, B_w_down)
        return out.reshape(b, s, d)
    return fn


@jax.jit
def pallas_parallel_sum__sliding_local_dilated__glu_gated_bilinear__prompt_kernel(
    A_x: jax.Array,
    A_wqkv: jax.Array,
    A_wo: jax.Array,
    B_x: jax.Array,
    B_w_gate: jax.Array,
    B_w_up: jax.Array,
    B_w_down: jax.Array,
):
    return make()(A_x, A_wqkv, A_wo, B_x, B_w_gate, B_w_up, B_w_down)
```

```python
import functools

import jax
import jax.numpy as jnp
import jax.experimental.pallas as pl
import jax.experimental.pallas.tpu as pltpu

F32, BF16, U32 = jnp.float32, jnp.bfloat16, jnp.uint32
HEAD_DIM, WINDOW, DILATION, EPS = 32, 8, 2, 1e-5
LANES, PAD = 128, 16

LHS = ((0, 1, 3), (2, 1, 3), (0, 0, 0), (3, 0, 3), (0, 1, 1), (2, -1, 0), (1, -1, 3))
RHS = ((0, 1, 3), (0, 0, 0), (1, -1, 3), (2, -1, 0), (3, 0, 3), (0, 1, 1), (2, 1, 3))
OUT = (((0, 1), (3, 1)), ((2, 1), (3, -1)), ((1, 1), (3, 1)), ((0, 1), (2, 1)),
       ((0, -1), (1, 1)), ((3, 1),), ((0, 1),))
ORDER = (1, 4, 3, 2, 0, 5, 6)
COMPLETES = {3: 2, 2: 1, 5: 3, 6: 0}
DOWN_ORDER = (3, 1, 6, 2, 4, 5, 0)


def _dot(a, b):
    return jnp.dot(a, b, preferred_element_type=F32)


def _comb(spec, quad):
    i, sign, j = spec
    return quad[i] if sign == 0 else quad[i] + quad[j] if sign > 0 else quad[i] - quad[j]


class _Quadrants:
    def __init__(self):
        self.val, self.sign = [None] * 4, [1] * 4

    def add(self, o, m):
        for q, s in OUT[o]:
            if self.val[q] is None:
                self.val[q], self.sign[q] = m, s
            elif self.sign[q] < 0:
                self.val[q], self.sign[q] = m - self.val[q], 1
            else:
                self.val[q] = self.val[q] + m if s > 0 else self.val[q] - m


def _recombine(product):
    c = _Quadrants()
    for o in ORDER:
        c.add(o, product(o))
    return c.val


def _pack(v):
    return pltpu.bitcast(v.astype(BF16), U32)


def _unpack(v):
    return pltpu.bitcast(v, BF16)


class _SideWork:
    def __init__(self, jobs, first, last, never):
        self.jobs, self.slots, self.done, self.n, self.never = jobs, last - first + 1, 0, -first, never

    def step(self, product):
        self.n += 1
        end = min(len(self.jobs), -(-len(self.jobs) * self.n // self.slots))
        todo = self.jobs[self.done:max(end, self.done)]
        self.done += len(todo)
        rows = product.shape[0] // 8
        for k, job in enumerate(todo):
            col, row = divmod(k * rows * (product.shape[1] // LANES) // len(todo), rows)
            tile = product[8 * row:8 * row + 8, col * LANES:(col + 1) * LANES]

            def after(v, tile=tile):
                if self.never is None:
                    return v
                t = tile if v.dtype == F32 else pltpu.bitcast(tile, v.dtype)
                return jnp.where(self.never, jnp.concatenate([t] * (v.shape[0] // 8), axis=0), v)

            job(after)


def _swap_block_lane(blocks):
    lane = jax.lax.broadcasted_iota(jnp.int32, blocks[0].shape, 1)
    t = [x if b == 0 else pltpu.roll(x, b, 1) for b, x in enumerate(blocks)]
    s = [t[(-c) % 8] for c in range(8)]
    for bit in (1, 2, 4):
        m = (lane & bit) != 0
        s = [jnp.where(m, s[(c - bit) % 8], s[c]) for c in range(8)]
    return [x if c == 0 else pltpu.roll(x, LANES - c, 1) for c, x in enumerate(s)]


def _attention(qkv_s, row, n, after):
    lane = jax.lax.broadcasted_iota(jnp.int32, (n, LANES), 1)
    pos = jax.lax.broadcasted_iota(jnp.int32, (n, LANES), 0) + row
    q = [after(qkv_s[0, c, pl.ds(row + PAD, n), :]) for c in range(8)]
    logits = []
    for w in range(WINDOW):
        rows = pl.ds(row + (PAD - DILATION * w), n)
        s = q[0] * qkv_s[1, 0, rows, :]
        for c in range(1, 8):
            s = s + q[c] * qkv_s[1, c, rows, :]
        s = s + pltpu.roll(s, LANES - 8, 1)
        s = s + pltpu.roll(s, LANES - 16, 1)
        s = s * (HEAD_DIM ** -0.5)
        if w:
            s = jnp.where(pos >= DILATION * w, s, -1e9)
        logits.append(s)
    m = functools.reduce(jnp.maximum, logits)
    e = [jnp.exp(s - m) for s in logits]
    inv = 1.0 / functools.reduce(lambda a, b: a + b, e)
    p = []
    for w in range(WINDOW):
        a = e[w] * inv
        a = jnp.where((lane & 24) == 0, a, pltpu.roll(a, 8, 1))
        a = jnp.where((lane & 16) == 0, a, pltpu.roll(a, 16, 1))
        p.append(a)
    out = []
    for c in range(8):
        o = p[0] * qkv_s[2, c, pl.ds(row + PAD, n), :]
        for w in range(1, WINDOW):
            o = o + p[w] * qkv_s[2, c, pl.ds(row + (PAD - DILATION * w), n), :]
        out.append(o)
    return _swap_block_lane(out)


def _kernel(x_hbm, wqkv_hbm, wo_hbm, wg_hbm, wu_hbm, wd_hbm, out_hbm,
            x_v, wqkv_v, wp_v, wo_v, wg_v, wu_v, wd_v, a1, a2, acc, qkv_s, stat,
            x_sem, w_sem, f_sem, o_sem, *, tf, nxg, nog, ahead, att, side2, perm, nsplit, down, pace, wos, zero):
    _, qm, d = x_v.shape
    hm, em, hd, qd, qf = 2 * qm, qm // 2, d // 2, d // 4, tf // 4
    nf = wg_hbm.shape[1] // tf
    xr, wr, orows = qm // nxg, d // nxg, qm // nog

    def first_copies(g):
        r = pl.ds(pl.multiple_of(g * xr, xr), xr)
        k = pl.ds(pl.multiple_of(g * wr, wr), wr)
        return (pltpu.make_async_copy(x_hbm.at[:, r, :], x_v.at[:, r, :], x_sem.at[0, g]),
                pltpu.make_async_copy(wqkv_hbm.at[k, pl.ds(0, d)], wqkv_v.at[0, k], x_sem.at[1, g]))

    def w_copy(m):
        cols = pl.ds(pl.multiple_of(m * d, d), d)
        return pltpu.make_async_copy(wqkv_hbm.at[:, cols], wqkv_v.at[m], w_sem.at[m])

    wo_copy = pltpu.make_async_copy(wo_hbm, wo_v, w_sem.at[0])

    def f_copies(j, slot):
        c = pl.ds(pl.multiple_of(j * tf, tf), tf)
        return (pltpu.make_async_copy(wg_hbm.at[:, c], wg_v.at[slot], f_sem.at[0, slot]),
                pltpu.make_async_copy(wu_hbm.at[:, c], wu_v.at[slot], f_sem.at[1, slot]),
                pltpu.make_async_copy(wd_hbm.at[c, :], wd_v.at[slot], f_sem.at[2, slot]))

    def o_copy(g):
        r = pl.ds(pl.multiple_of(g * orows, orows), orows)
        return pltpu.make_async_copy(x_v.at[:, r, :], out_hbm.at[:, r, :], o_sem.at[g])

    for g in range(ahead):
        for c in first_copies(g):
            c.start()

    def permute_weight(m, r0, n, after=lambda v: v):
        hint = (lambda v, k: v) if isinstance(r0, int) else pl.multiple_of
        blocks = [pltpu.bitcast(wqkv_v[m, pl.ds(hint(r0, n), n), b * LANES:(b + 1) * LANES], U32) for b in range(8)]
        for c, v in enumerate(_swap_block_lane([after(v) for v in blocks])):
            wp_v[m, pl.ds(hint(r0 // 2, n // 2), n // 2), c * LANES:(c + 1) * LANES] = v

    def first_level(o, a, b, r0, n):
        return 4 * o + b + 2 * (r0 // em), pl.ds(pl.multiple_of(r0 % em + a * em, 16), n)

    def ln_body(g, carry):
        for c in first_copies(g):
            c.wait()

        @pl.when(g + ahead < nxg)
        def _():
            for c in first_copies(g + ahead):
                c.start()

        @pl.when(g + ahead == nxg)
        def _():
            w_copy(1).start()

        permute_weight(0, g * wr, wr)
        for n in range(0, xr, 16):
            r0 = pl.multiple_of(g * xr + n, 16)
            blk = []
            for q in range(4):
                x = x_v[q, pl.ds(r0, 16), :].astype(F32)
                mean = jnp.mean(x, axis=-1, keepdims=True)
                xc = x - mean
                rstd = jax.lax.rsqrt(jnp.mean(xc * xc, axis=-1, keepdims=True) + EPS)
                stat[0, q, pl.ds(r0, 16), :] = jnp.broadcast_to(mean, (16, LANES))
                stat[1, q, pl.ds(r0, 16), :] = jnp.broadcast_to(rstd, (16, LANES))
                xn = xc * rstd
                blk.append([xn[:, p * qd:(p + 1) * qd] for p in range(4)])
            for a in range(2):
                for b in range(2):
                    quad = [blk[a + 2 * i][b + 2 * k] for i in range(2) for k in range(2)]
                    for o in range(7):
                        a1[first_level(o, a, b, r0, 16)] = _comb(LHS[o], quad).astype(BF16)
        return carry

    jax.lax.fori_loop(0, nxg, ln_body, 0)

    side = -(-qm // (16 * 6))

    def qkv_body(t, carry):
        m, half = t // 2, t % 2

        @pl.when(jnp.logical_and(half == 1, m < 2))
        def _():
            w_copy(m + 1).wait()

        @pl.when(t == 1)
        def _():
            w_copy(2).start()

        @pl.when(t == 3)
        def _():
            for c in f_copies(0, 0):
                c.start()
            wo_copy.start()

        base = jnp.minimum(t * (16 * side), qm - 16 * side)

        blk = {}

        def second_level(n, p, o, after):
            r0 = pl.multiple_of(base + 16 * n, 16)
            r = pl.ds(r0, 16)
            if o < 0:
                mean = [after(stat[0, q, r, :]) for q in range(4)]
                blk[n, p] = [[(x_v[q, r, k * qd + p:k * qd + p + LANES].astype(F32) - mean[q]) * stat[1, q, r, :]
                              for k in range(4)] for q in range(4)]
                return
            quad = [after(_comb(LHS[o], [blk[n, p][a + 2 * i][b + 2 * k] for i in range(2) for k in range(2)]))
                    for a in range(2) for b in range(2)]
            for i in range(7):
                a2[7 * o + i, pl.ds(pl.multiple_of(r0 // 2, 8), 8), p:p + LANES] = _pack(_comb(LHS[i], quad))

        def clear(k, after):
            zero = after(jnp.zeros((8, LANES), F32))
            acc[k, pl.ds(pl.multiple_of(base, 16), 16 * side), :] = jnp.tile(zero, (2 * side, qd // LANES))

        work = [_SideWork([functools.partial(clear, k) for k in range(49)], *zero, t >= 6),
                _SideWork([functools.partial(second_level, n, p, o)
                           for n in range(side) for p in (0, LANES) for o in range(-1, 7)], *side2,
                          t >= 6 if "s" in pace else None),
                _SideWork([functools.partial(permute_weight, jnp.minimum((t + 1) // 2, 2), n, perm[2])
                           for n in range(0, d, perm[2])], *perm[:2], t >= 6 if "p" in pace else None)]
        nw = hd // nsplit

        weights = {n: [_unpack(wp_v[m, i * qd:(i + 1) * qd, k * hd + n:k * hd + n + nw]).astype(F32)
                       for i in range(2) for k in range(2)] for n in range(0, hd, nw)}

        def product(o, n):
            w = weights[n]
            lhs = jnp.concatenate([a1[4 * o + b + 2 * half] for b in range(2)], axis=1)
            p = _dot(lhs, _comb(RHS[o], w).astype(BF16))
            for s in work:
                s.step(p)
            return p

        for n in range(0, hd, nw):
            c = _Quadrants()
            for o in ORDER:
                c.add(o, product(o, n))
                if o in COMPLETES:
                    i, b = divmod(COMPLETES[o], 2)
                    for a in range(2):
                        dst = pl.ds(pl.multiple_of(PAD + (2 * i + a) * qm + half * em, 8), em)
                        for p in range(0, nw, LANES):
                            qkv_s[m, 4 * b + (n + p) // LANES, dst, :] = (
                                c.val[COMPLETES[o]][a * em:(a + 1) * em, p:p + LANES])
        return carry

    jax.lax.fori_loop(0, 6, qkv_body, 0)
    for m in (1, 2):
        for c in range(8):
            qkv_s[m, c, :PAD, :] = jnp.broadcast_to(qkv_s[m, c, PAD:PAD + 1, :], (PAD, LANES))

    wo_copy.wait()

    def wo_operand(o, r0, n):
        return o // 4, pl.ds(r0 // 2 + o // 2 % 2 * qd, n // 2), slice(o % 2 * hd, (o % 2 + 1) * hd)

    groups = -(-hm // (16 * nf))

    def ffn_body(j, carry):
        slot = j % 2

        @pl.when(j + 1 < nf)
        def _():
            for c in f_copies(j + 1, 1 - slot):
                c.start()

        for c in f_copies(j, slot):
            c.wait()

        base = jnp.minimum(j * (16 * groups), hm - 16 * groups)
        top = {}

        def attend(n, bottom, after):
            r0 = pl.multiple_of(base + 16 * n, 16)
            if not bottom:
                top[n] = _attention(qkv_s, r0, 16, after)
                return
            bot = _attention(qkv_s, r0 + hm, 16, after)
            for p in range(4):
                quad = (top[n][p], top[n][p + 4], bot[p], bot[p + 4])
                cols = slice(p % 2 * LANES, (p % 2 + 1) * LANES)
                for o in range(7):
                    a1[first_level(o, r0 // qm, p // 2, r0 % qm, 16) + (cols,)] = _comb(LHS[o], quad).astype(BF16)

        work = _SideWork([functools.partial(attend, n, b) for n in range(groups) for b in range(2)], *att,
                         j >= nf if "a" in pace else None)

        wo_groups = -(-hd // (16 * nf))

        def split_wo(n, p, after):
            r0 = jnp.minimum(j * (16 * wo_groups), hd - 16 * wo_groups) + 16 * n
            wo = [after(wo_v[pl.ds(pl.multiple_of(r0 + i * hd, 16), 16), k * hd + p:k * hd + p + LANES].astype(F32))
                  for i in range(2) for k in range(2)]
            for o in range(7):
                m, r, c = wo_operand(o, r0, 16)
                wp_v[m, pl.ds(pl.multiple_of(r.start, 8), 8), c.start + p:c.start + p + LANES] = (
                    _pack(_comb(RHS[o], wo)))

        wo_work = _SideWork([functools.partial(split_wo, n, p) for n in range(wo_groups) for p in range(0, hd, LANES)],
                            *wos, j >= nf)

        def in_block(i, k):
            r, c = slice(i * qd, (i + 1) * qd), slice(k * qf, (k + 1) * qf)
            return jnp.concatenate([wg_v[slot, r, c].astype(F32), wu_v[slot, r, c].astype(F32)], axis=1)

        def out_block(i, k):
            return wd_v[slot, i * qf:(i + 1) * qf, k * qd:(k + 1) * qd].astype(F32)

        def quadrants(block):
            return [[block(a + 2 * i, b + 2 * k) for i in range(2) for k in range(2)]
                    for a in range(2) for b in range(2)]

        w_in, w_out = quadrants(in_block), quadrants(out_block)
        gu = [_Quadrants() for _ in range(4)]
        h = [[None] * 4 for _ in range(4)]
        for o in ORDER:
            rhs = [_comb(RHS[o], w) for w in w_in]

            def product(i):
                p = _dot(_unpack(a2[7 * o + i]), _comb(RHS[i], rhs).astype(BF16))
                work.step(p)
                wo_work.step(p)
                return p

            for s, v in enumerate(_recombine(product)):
                gu[s].add(o, v)
                if o in COMPLETES:
                    q = COMPLETES[o]
                    h[s][q] = gu[s].val[q][:, :qf] * gu[s].val[q][:, qf:]
        for o in down[0]:
            lhs = [_comb(LHS[o], v) for v in h]
            rhs = [_comb(RHS[o], w) for w in w_out]
            for i in down[1]:
                p = _dot(_comb(LHS[i], lhs).astype(BF16), _comb(RHS[i], rhs).astype(BF16))
                acc[7 * o + i] += p
                work.step(p)
                wo_work.step(p)
        return carry

    jax.lax.fori_loop(0, nf, ffn_body, 0)

    def out_body(g, carry):
        r0 = pl.multiple_of(g * orows, orows)
        r = pl.ds(r0, orows)
        res = [_Quadrants() for _ in range(4)]
        for o in ORDER:
            lhs = jnp.concatenate([jnp.concatenate([a1[first_level(o, a, b, r0, orows)]
                                                    for b in range(2)], axis=1) for a in range(2)], axis=0)
            p = _dot(lhs, _unpack(wp_v[wo_operand(o, 0, hd)]))
            c = _recombine(lambda i: acc[7 * o + i, r, :])
            for s in range(4):
                a, b = divmod(s, 2)
                res[s].add(o, p[a * orows:(a + 1) * orows, b * qd:(b + 1) * qd] + c[s])
                if o in COMPLETES:
                    i, k = divmod(COMPLETES[o], 2)
                    cols = slice((b + 2 * k) * qd, (b + 2 * k + 1) * qd)
                    x = x_v[a + 2 * i, r, cols].astype(F32)
                    x_v[a + 2 * i, r, cols] = (x + res[s].val[COMPLETES[o]]).astype(BF16)
        o_copy(g).start()
        return carry

    jax.lax.fori_loop(0, nog, out_body, 0)
    for g in range(nog):
        o_copy(g).wait()


EVEN = {"XLA_TPU_EVENLY_DISTRIBUTE_CRITICAL_NODES": True}


def make(tf=512, nxg=16, nog=4, ahead=3, att=(0, 89), side2=(0, 4), perm=(1, 5, 32), nsplit=1, down=(DOWN_ORDER, (2, 3, 1, 6, 4, 5, 0)), pace="sp", wos=(3, 30), zero=(0, 5), flags=EVEN):
    def fn(A_x, A_wqkv, A_wo, B_x, B_w_gate, B_w_up, B_w_down):
        del B_x
        b, s, d = A_x.shape
        qm = s // 4
        any_spec = pl.BlockSpec(memory_space=pl.ANY)
        out = pl.pallas_call(
            functools.partial(_kernel, tf=tf, nxg=nxg, nog=nog, ahead=ahead, att=att, side2=side2, perm=perm,
                              nsplit=nsplit, down=down, pace=pace, wos=wos, zero=zero),
            in_specs=[any_spec] * 6,
            out_specs=any_spec,
            out_shape=jax.ShapeDtypeStruct((4, qm, d), A_x.dtype),
            scratch_shapes=[
                pltpu.VMEM((4, qm, d), BF16),
                pltpu.VMEM((3, d, d), BF16),
                pltpu.VMEM((3, d // 2, d), U32),
                pltpu.VMEM((d, d), BF16),
                pltpu.VMEM((2, d, tf), BF16),
                pltpu.VMEM((2, d, tf), BF16),
                pltpu.VMEM((2, tf, d), BF16),
                pltpu.VMEM((28, qm, d // 4), BF16),
                pltpu.VMEM((49, qm // 2, d // 4), U32),
                pltpu.VMEM((49, qm, d // 4), F32),
                pltpu.VMEM((3, 8, PAD + s, LANES), F32),
                pltpu.VMEM((2, 4, qm, LANES), F32),
                pltpu.SemaphoreType.DMA((2, nxg)),
                pltpu.SemaphoreType.DMA((3,)),
                pltpu.SemaphoreType.DMA((3, 2)),
                pltpu.SemaphoreType.DMA((nog,)),
            ],
            compiler_params=pltpu.CompilerParams(vmem_limit_bytes=126 * 2 ** 20, flags=flags),
        )(A_x.reshape(4, qm, d), A_wqkv, A_wo, B_w_gate, B_w_up, B_w_down)
        return out.reshape(b, s, d)
    return fn


@jax.jit
def pallas_parallel_sum__sliding_local_dilated__glu_gated_bilinear__prompt_kernel(
    A_x: jax.Array,
    A_wqkv: jax.Array,
    A_wo: jax.Array,
    B_x: jax.Array,
    B_w_gate: jax.Array,
    B_w_up: jax.Array,
    B_w_down: jax.Array,
):
    return make(zero=(4,5), ahead=5)(A_x, A_wqkv, A_wo, B_x, B_w_gate, B_w_up, B_w_down)
```

```python
import functools

import jax
import jax.numpy as jnp
import jax.experimental.pallas as pl
import jax.experimental.pallas.tpu as pltpu

F32, BF16, U32 = jnp.float32, jnp.bfloat16, jnp.uint32
HEAD_DIM, WINDOW, DILATION, EPS = 32, 8, 2, 1e-5
LANES, PAD = 128, 16

LHS = ((0, 1, 3), (2, 1, 3), (0, 0, 0), (3, 0, 3), (0, 1, 1), (2, -1, 0), (1, -1, 3))
RHS = ((0, 1, 3), (0, 0, 0), (1, -1, 3), (2, -1, 0), (3, 0, 3), (0, 1, 1), (2, 1, 3))
ORDER = (1, 4, 0, 3, 2, 6, 5)
COMPLETES = {3: 2, 2: 1, 5: 3, 6: 0}
DOWN_ORDER = (2, 4, 5, 3, 1, 6, 0)


def _dot(a, b):
    return jnp.dot(a, b, preferred_element_type=F32)


def _comb(spec, quad):
    i, sign, j = spec
    return quad[i] if sign == 0 else quad[i] + quad[j] if sign > 0 else quad[i] - quad[j]


def _lazy_comb(spec, get):
    i, sign, j = spec
    return get(i) if sign == 0 else get(i) + get(j) if sign > 0 else get(i) - get(j)


class _Quadrants:
    def __init__(self, slots=None):
        self.slots = {} if slots is None else slots

    def add(self, o, m):
        t, done = self.slots, None
        if o == 1:
            t[0] = m
        elif o == 4:
            t[1] = m
        elif o == 3:
            done = t[0] + m
            t[2] = m - t[1]
        elif o == 2:
            done = m + t[1]
            t[3] = m - t[0]
        elif o == 0:
            t[4] = m
        else:
            done = t[3 if o == 5 else 2] + t[4] + m
        return done


class _Parked:
    def __init__(self, refs, zero, rows):
        self.refs, self.rows = refs, rows
        self.again = pl.ds(0 if isinstance(zero, int) else pl.multiple_of(zero * 8, 8), rows)

    def __setitem__(self, k, v):
        self.refs[k][:self.rows, :v.shape[1]] = v
        self.cols = v.shape[1]

    def __getitem__(self, k):
        return self.refs[k][self.again, :self.cols]


def _recombine(product):
    c = _Quadrants()
    done = {COMPLETES.get(o): c.add(o, product(o)) for o in ORDER}
    return [done[q] for q in range(4)]


def _pack(v):
    return pltpu.bitcast(v.astype(BF16), U32)


def _unpack(v):
    return pltpu.bitcast(v, BF16)


class _SideWork:
    def __init__(self, jobs, first, last, never):
        self.jobs, self.slots, self.done, self.n, self.never = jobs, last - first + 1, 0, -first, never

    def step(self, product):
        self.n += 1
        end = min(len(self.jobs), -(-len(self.jobs) * self.n // self.slots))
        todo = self.jobs[self.done:max(end, self.done)]
        self.done += len(todo)
        rows = product.shape[0] // 8
        for k, job in enumerate(todo):
            col, row = divmod(k * rows * (product.shape[1] // LANES) // len(todo), rows)
            tile = product[8 * row:8 * row + 8, col * LANES:(col + 1) * LANES]

            def after(v, tile=tile):
                if self.never is None:
                    return v
                t = tile if v.dtype == F32 else pltpu.bitcast(tile, v.dtype)
                return jnp.where(self.never, jnp.concatenate([t] * (v.shape[0] // 8), axis=0), v)

            job(after)


def _swap_block_lane(blocks):
    lane = jax.lax.broadcasted_iota(jnp.int32, blocks[0].shape, 1)
    t = [x if b == 0 else pltpu.roll(x, b, 1) for b, x in enumerate(blocks)]
    s = [t[(-c) % 8] for c in range(8)]
    for bit in (1, 2, 4):
        m = (lane & bit) != 0
        s = [jnp.where(m, s[(c - bit) % 8], s[c]) for c in range(8)]
    return [x if c == 0 else pltpu.roll(x, LANES - c, 1) for c, x in enumerate(s)]


def _attention(qkv_s, row, n, after):
    lane = jax.lax.broadcasted_iota(jnp.int32, (n, LANES), 1)
    pos = jax.lax.broadcasted_iota(jnp.int32, (n, LANES), 0) + row
    q = [after(qkv_s[0, c, pl.ds(row + PAD, n), :]) for c in range(8)]
    logits = []
    for w in range(WINDOW):
        rows = pl.ds(row + (PAD - DILATION * w), n)
        s = q[0] * qkv_s[1, 0, rows, :]
        for c in range(1, 8):
            s = s + q[c] * qkv_s[1, c, rows, :]
        s = s + pltpu.roll(s, LANES - 8, 1)
        s = s + pltpu.roll(s, LANES - 16, 1)
        s = s * (HEAD_DIM ** -0.5)
        if w:
            s = jnp.where(pos >= DILATION * w, s, -1e9)
        logits.append(s)
    m = functools.reduce(jnp.maximum, logits)
    e = [jnp.exp(s - m) for s in logits]
    inv = 1.0 / functools.reduce(lambda a, b: a + b, e)
    p = []
    for w in range(WINDOW):
        a = e[w] * inv
        a = jnp.where((lane & 24) == 0, a, pltpu.roll(a, 8, 1))
        a = jnp.where((lane & 16) == 0, a, pltpu.roll(a, 16, 1))
        p.append(a)
    out = []
    for c in range(8):
        o = p[0] * qkv_s[2, c, pl.ds(row + PAD, n), :]
        for w in range(1, WINDOW):
            o = o + p[w] * qkv_s[2, c, pl.ds(row + (PAD - DILATION * w), n), :]
        out.append(o)
    return _swap_block_lane(out)


def _kernel(x_hbm, wqkv_hbm, wo_hbm, wg_hbm, wu_hbm, wd_hbm, out_hbm,
            x_v, wqkv_v, wp_v, ws_v, wo_v, wg_v, wu_v, wd_v, a1, a2, acc, qkv_s, stat, tmp, hid,
            x_sem, w_sem, f_sem, o_sem, *, tf, nxg, nog, ahead, att, side2, perm, norm, down, pace, wos, zero, otmp, park, staged, an):
    _, qm, d = x_v.shape
    hm, em, hd, qd, qf = 2 * qm, qm // 2, d // 2, d // 4, tf // 4
    nf = wg_hbm.shape[1] // tf
    br = qm // 4
    xr, wr, orows = br // nxg, hd // nxg, qm // nog

    def first_copies(g):
        r = pl.ds(pl.multiple_of(g * xr, xr), xr)
        k = pl.ds(pl.multiple_of(g * wr, wr), wr)
        return (pltpu.make_async_copy(wqkv_hbm.at[:, k, pl.ds(0, d)], wqkv_v.at[0, :, k], x_sem.at[1, g]),
                pltpu.make_async_copy(x_hbm.at[:, r, :], x_v.at[:, r, :], x_sem.at[0, g]))

    def x_copy(g):
        r = pl.ds(pl.multiple_of(g * br, br), br)
        return pltpu.make_async_copy(x_hbm.at[:, r, :], x_v.at[:, r, :], w_sem.at[2 + g])

    def w_copy(m):
        cols = pl.ds(pl.multiple_of(m * d, d), d)
        return pltpu.make_async_copy(wqkv_hbm.at[:, :, cols], wqkv_v.at[m], w_sem.at[m])

    wo_copy = pltpu.make_async_copy(wo_hbm, wo_v, w_sem.at[0])

    def f_copies(j, slot):
        c = pl.ds(pl.multiple_of(j * tf, tf), tf)
        return (pltpu.make_async_copy(wg_hbm.at[:, c], wg_v.at[slot], f_sem.at[0, slot]),
                pltpu.make_async_copy(wu_hbm.at[:, c], wu_v.at[slot], f_sem.at[1, slot]),
                pltpu.make_async_copy(wd_hbm.at[c, :], wd_v.at[slot], f_sem.at[2, slot]))

    def o_copy(t, k):
        at = (slice(None), pl.ds(pl.multiple_of(t // 2 * orows, orows), orows),
              pl.ds(pl.multiple_of(t % 2 * qd + k * hd, qd), qd))
        return pltpu.make_async_copy(x_v.at[at], out_hbm.at[at], o_sem.at[k, t])

    for g in range(min(ahead, nxg)):
        for c in first_copies(g):
            c.start()

    def permuted_weight(m, i, r0, n, after=lambda v: v):
        hint = (lambda v, k: v) if isinstance(r0, int) else pl.multiple_of
        return _swap_block_lane([after(pltpu.bitcast(wqkv_v[m, i, pl.ds(hint(r0, n), n), c:c + LANES], U32))
                                 for c in range(0, d, LANES)])

    def first_level(o, a, b, r0, n):
        return b + 2 * (r0 // em), pl.ds(pl.multiple_of(r0 % em + a * em, min(n, 16)), n)

    def staged_operand(o, n, r0, a, after):
        for c in range(0, hd, LANES):
            v = _lazy_comb(LHS[o], lambda q: tmp[q // 2 * 4 + (q % 2 * hd + c) // qd][
                pl.ds(pl.multiple_of(r0 // qm * 8 + a * br + n, 8), 32), c % qd:c % qd + LANES])
            a1[o][first_level(o, a, c // qd, r0 + n, 32) + (slice(c % qd, c % qd + LANES),)] = after(v).astype(BF16)

    def layer_norm(r0, a, after=lambda v: v, n=None):
        r = pl.ds(r0, 16)
        xn = []
        for q in (a, a + 2):
            x = [after(x_v[q, r, c:c + LANES].astype(F32)) for c in range(0, d, LANES)]
            mean = jnp.sum(functools.reduce(jnp.add, x), axis=-1, keepdims=True) * (1.0 / d)
            x = [v - mean for v in x]
            var = jnp.sum(functools.reduce(jnp.add, [v * v for v in x]), axis=-1, keepdims=True) * (1.0 / d)
            rstd = jax.lax.rsqrt(var + EPS)
            stat[0, q, r, :] = jnp.broadcast_to(mean, (16, LANES))
            stat[1, q, r, :] = jnp.broadcast_to(rstd, (16, LANES))
            xn.append([v * rstd for v in x])
        if n is not None:
            for i in range(2):
                for p in range(8):
                    tmp[i * 4 + p // 2][a * br + n:a * br + n + 16, p % 2 * LANES:(p % 2 + 1) * LANES] = xn[i][p]
            return
        for p in range(4):
            quad = (xn[0][p], xn[0][p + 4], xn[1][p], xn[1][p + 4])
            cols = slice(p % 2 * LANES, (p % 2 + 1) * LANES)
            for o in range(7):
                a1[o][first_level(o, a, p // 2, r0, 16) + (cols,)] = _comb(LHS[o], quad).astype(BF16)

    def store_split(r0, n, p, quad):
        for o in range(7):
            ws_v[2 * o + p // qd, pl.ds(pl.multiple_of(r0 // 2, 8), n // 2), p % qd:p % qd + LANES] = (
                _pack(_comb(RHS[o], quad)))

    def ln_body(g, carry):
        for c in first_copies(g):
            c.wait()

        @pl.when(g + ahead < nxg)
        def _():
            for c in first_copies(g + ahead):
                c.start()

        @pl.when(g == max(nxg - ahead, 0))
        def _():
            x_copy(1).start()

        w = [[_unpack(v).astype(F32) for v in permuted_weight(0, i, g * wr, wr)] for i in range(2)]
        for p in range(4):
            store_split(g * wr, wr, p * LANES, (w[0][p], w[0][p + 4], w[1][p], w[1][p + 4]))
        for n in range(0, xr, 16):
            for a in range(2):
                layer_norm(pl.multiple_of(g * xr + n, 16), a)
        return carry

    jax.lax.fori_loop(0, nxg, ln_body, 0)

    def store_projection(m, q, r0, n, c0, v):
        for a in range(2):
            dst = pl.ds(pl.multiple_of(PAD + (q // 2 * 2 + a) * qm + r0, 8), n)
            for p in range(0, v.shape[1], LANES):
                qkv_s[m, q % 2 * 4 + (c0 + p) // LANES, dst, :] = v[a * n:(a + 1) * n, p:p + LANES]

    def first_level_rows(o, r0, n, order=(0, 1)):
        return jnp.concatenate([jnp.concatenate([a1[o][first_level(o, a, b, r0, n)] for b in range(2)], axis=1)
                                for a in order], axis=0)

    def q_body(g, carry):
        @pl.when(g < 2)
        def _():
            x_copy(g + 2).start()
            w_copy(g + 1).start()

        pl.when(g == 2)(wo_copy.start)

        @pl.when(g < 3)
        def _():
            x_copy(g + 1).wait()

        @pl.when(g >= 2)
        def _():
            w_copy(g - 1).wait()

        def permute(i, n, after):
            for c, v in enumerate(permuted_weight(jnp.maximum(g - 1, 0), i, n, perm[2], after)):
                wp_v[g // 3, (i * hd + n) // 2:(i * hd + n + perm[2]) // 2, c * LANES:(c + 1) * LANES] = v

        nxt = (g + 1) % 4 * br
        work = [_SideWork([functools.partial(layer_norm, pl.multiple_of(nxt + n, 16), a, n=n if staged else None)
                           for n in range(0, br, 16) for a in range(2)], *norm, g >= 4 if "n" in pace else None),
                _SideWork([functools.partial(permute, i, n) for i in range(2) for n in range(0, hd, perm[2])],
                          *perm[:2], g >= 4 if "p" in pace else None)]
        if staged:
            work.append(_SideWork([functools.partial(staged_operand, o, n, nxt, a) for o in ORDER
                                   for n in range(0, br, 32) for a in range(2)], *staged, g >= 4))
        r0 = pl.multiple_of(g * br, br)
        lhs = {o: first_level_rows(o, r0, br) for o in ORDER}
        c = _Quadrants()
        for o in ORDER:
            p = _dot(lhs[o], jnp.concatenate([_unpack(ws_v[2 * o + b]) for b in range(2)], axis=1))
            for s in work:
                s.step(p)
            done = c.add(o, p)
            if done is not None:
                store_projection(0, COMPLETES[o], r0, br, 0, done)
        return carry

    jax.lax.fori_loop(0, 4, q_body, 0)
    for c in f_copies(0, 0):
        c.start()
    wo_copy.wait()

    side = qm // (16 * 4)

    def kv_body(t, carry):
        m, half = t // 2, t % 2
        base = t * (16 * side)
        blk = {}

        def second_level(n, p, o, after):
            r0 = pl.multiple_of(base + 16 * n, 16)
            r = pl.ds(r0, 16)
            if o < 0:
                mean = [after(stat[0, q, r, :]) for q in range(4)]
                blk[n, p] = [[(x_v[q, r, k * qd + p:k * qd + p + LANES].astype(F32) - mean[q]) * stat[1, q, r, :]
                              for k in range(4)] for q in range(4)]
                return
            quad = [after(_comb(LHS[o], [blk[n, p][a + 2 * i][b + 2 * k] for i in range(2) for k in range(2)]))
                    for a in range(2) for b in range(2)]
            for i in range(7):
                a2[7 * o + i, pl.ds(pl.multiple_of(r0 // 2, 8), 8), p:p + LANES] = _pack(_comb(LHS[i], quad))

        def clear(k, after):
            zero = after(jnp.zeros((8, LANES), F32))
            acc[k, pl.ds(pl.multiple_of(base, 16), 16 * side), :] = jnp.tile(zero, (2 * side, qd // LANES))

        def split_wo(n, p, after):
            r0 = t * (hd // 4) + n
            store_split(r0, 16, p, [
                after(wo_v[pl.ds(pl.multiple_of(r0 + i, 16), 16), k + p:k + p + LANES].astype(F32))
                for i in (0, hd) for k in (0, hd)])

        work = [_SideWork([functools.partial(split_wo, n, p)
                           for n in range(0, hd // 4, 16) for p in range(0, hd, LANES)], *wos, t >= 4),
                _SideWork([functools.partial(clear, k) for k in range(49)], *zero, t >= 4),
                _SideWork([functools.partial(second_level, n, p, o)
                           for n in range(side) for p in (0, LANES) for o in range(-1, 7)], *side2, t >= 4)]
        w = [_unpack(wp_v[m, i * qd:(i + 1) * qd, k * hd:(k + 1) * hd]).astype(F32)
             for i in range(2) for k in range(2)]
        c = _Quadrants()
        for o in ORDER:
            lhs = jnp.concatenate([a1[o][b + 2 * half] for b in range(2)], axis=1)
            p = _dot(lhs, _comb(RHS[o], w).astype(BF16))
            for s in work:
                s.step(p)
            done = c.add(o, p)
            if done is not None:
                store_projection(m + 1, COMPLETES[o], half * em, em, 0, done)
        return carry

    jax.lax.fori_loop(0, 4, kv_body, 0)
    for m in (1, 2):
        for c in range(8):
            qkv_s[m, c, :PAD, :] = jnp.broadcast_to(qkv_s[m, c, PAD:PAD + 1, :], (PAD, LANES))

    groups = -(-hm // (an * nf))

    def ffn_body(j, carry):
        slot = j % 2

        @pl.when(j + 1 < nf)
        def _():
            for c in f_copies(j + 1, 1 - slot):
                c.start()

        for c in f_copies(j, slot):
            c.wait()

        base = jnp.minimum(j * (an * groups), hm - an * groups)
        top = {}

        def attend(n, bottom, after):
            r0 = pl.multiple_of(base + an * n, an)
            if not bottom:
                top[n] = _attention(qkv_s, r0, an, after)
                return
            bot = _attention(qkv_s, r0 + hm, an, after)
            for p in range(4):
                quad = (top[n][p], top[n][p + 4], bot[p], bot[p + 4])
                cols = slice(p % 2 * LANES, (p % 2 + 1) * LANES)
                for o in range(7):
                    a1[o][first_level(o, r0 // qm, p // 2, r0 % qm, an) + (cols,)] = _comb(LHS[o], quad).astype(BF16)

        work = _SideWork([functools.partial(attend, n, b) for n in range(groups if att[0] >= 0 else 0) for b in range(2)], *att,
                         j >= nf if "a" in pace else None)

        def w_in(s, q):
            i, k = s // 2 + q // 2 * 2, s % 2 + q % 2 * 2
            r, c = slice(i * qd, (i + 1) * qd), slice(k * qf, (k + 1) * qf)
            return jnp.concatenate([wg_v[slot, r, c].astype(F32), wu_v[slot, r, c].astype(F32)], axis=1)

        def w_out(s, q):
            i, k = s // 2 + q // 2 * 2, s % 2 + q % 2 * 2
            return wd_v[slot, i * qf:(i + 1) * qf, k * qd:(k + 1) * qd].astype(F32)

        def two_level(spec, o, i, get):
            return _lazy_comb(spec[i], lambda s: _lazy_comb(spec[o], lambda q: get(s, q))).astype(BF16)

        inner = _Quadrants(_Parked(tmp, j // nf, qm) if "i" in park else None)
        h = _Parked(hid, j // nf if "h" in park else 0, qm)
        outer = [_Quadrants(_Parked(tmp[5 * s + 5:], j // nf, qm) if "o" in park else None) for s in range(4)]
        for o in ORDER:
            for i in ORDER:
                p = _dot(_unpack(a2[7 * o + i]), two_level(RHS, o, i, w_in))
                v = inner.add(i, p)
                if v is not None:
                    gu = outer[COMPLETES[i]].add(o, v)
                    if gu is not None:
                        h[4 * COMPLETES[i] + COMPLETES[o]] = gu[:, :qf] * gu[:, qf:]
                work.step(p)
        for o in down[0]:
            for i in down[1]:
                p = _dot(two_level(LHS, o, i, lambda s, q: h[4 * s + q]), two_level(RHS, o, i, w_out))
                acc[7 * o + i] += p
                work.step(p)
        return carry

    if park != 'skip':
        jax.lax.fori_loop(0, nf, ffn_body, 0)
    else:
        ws_v[0] = a2[3]

    def out_body(t, carry):
        b = t % 2
        r0 = pl.multiple_of(t // 2 * orows, orows)
        r = pl.ds(r0, orows)
        res = [_Quadrants(), _Quadrants()]
        for o in ORDER:
            p = _dot(first_level_rows(o, r0, orows, (b, 1 - b)), _unpack(ws_v[2 * o + b]))
            shared = acc[7 * o + 3 - b, r, :]
            ffn = (shared - acc[7 * o + 4 - 3 * b, r, :] + acc[7 * o, r, :] + acc[7 * o + 6 - b, r, :],
                   shared + acc[7 * o + 1 + 3 * b, r, :])
            for s, a in enumerate((b, 1 - b)):
                done = res[s].add(o, p[s * orows:(s + 1) * orows] + ffn[s])
                if done is not None:
                    i, k = divmod(COMPLETES[o], 2)
                    at = (a + 2 * i, r, pl.ds(pl.multiple_of(b * qd + k * hd, qd), qd))
                    x_v[at] = (x_v[at].astype(F32) + done).astype(BF16)
        for k in range(2):
            o_copy(t, k).start()
        return carry

    jax.lax.fori_loop(0, 2 * nog, out_body, 0)
    for t in range(2 * nog):
        for k in range(2):
            o_copy(t, k).wait()


EVEN = {"XLA_TPU_EVENLY_DISTRIBUTE_CRITICAL_NODES": True}


def make(tf=512, nxg=4, nog=4, ahead=4, att=(0, 89), side2=(0, 5), perm=(0, 5, 32), norm=(0, 3), down=(DOWN_ORDER, (3, 2, 4, 5, 1, 6, 0)), pace="np", wos=(0, 5), zero=(0, 1), otmp=False, park="ioh", staged=(5, 6), flags=EVEN, nb=True, an=16):
    def fn(A_x, A_wqkv, A_wo, B_x, B_w_gate, B_w_up, B_w_down):
        del B_x
        b, s, d = A_x.shape
        qm = s // 4
        any_spec = pl.BlockSpec(memory_space=pl.ANY)
        out = pl.pallas_call(
            functools.partial(_kernel, tf=tf, nxg=nxg, nog=nog, ahead=ahead, att=att, side2=side2, perm=perm,
                              norm=norm, down=down, pace=pace, wos=wos, zero=zero, otmp=otmp, park=park, staged=staged, an=an),
            in_specs=[any_spec] * 6,
            out_specs=any_spec,
            out_shape=jax.ShapeDtypeStruct((4, qm, d), A_x.dtype),
            scratch_shapes=[
                pltpu.VMEM((4, qm, d), BF16),
                pltpu.VMEM((3, 2, d // 2, d), BF16),
                pltpu.VMEM((2, d // 2, d), U32),
                pltpu.VMEM((14, d // 4, d // 4), U32),
                pltpu.VMEM((d, d), BF16),
                pltpu.VMEM((2, d, tf), BF16),
                pltpu.VMEM((2, d, tf), BF16),
                pltpu.VMEM((2, tf, d), BF16),
                [pltpu.VMEM((4, qm, d // 4), BF16)] * 7,
                pltpu.VMEM((49, qm // 2, d // 4), U32),
                pltpu.VMEM((49, qm, d // 4), F32),
                pltpu.VMEM((3, 8, PAD + s, LANES), F32),
                pltpu.VMEM((2, 4, qm, LANES), F32),
                [pltpu.VMEM((qm, tf // 2), F32)] * 25,
                [pltpu.VMEM((qm, tf // 4), F32)] * 16,
                pltpu.SemaphoreType.DMA((2, nxg)),
                pltpu.SemaphoreType.DMA((6,)),
                pltpu.SemaphoreType.DMA((3, 2)),
                pltpu.SemaphoreType.DMA((2, 2 * nog)),
            ],
            compiler_params=pltpu.CompilerParams(vmem_limit_bytes=126 * 2 ** 20, flags=flags, disable_bounds_checks=nb),
        )(A_x.reshape(4, qm, d), A_wqkv.reshape(2, d // 2, 3 * d), A_wo, B_w_gate, B_w_up, B_w_down)
        return out.reshape(b, s, d)
    return fn


@jax.jit
def pallas_parallel_sum__sliding_local_dilated__glu_gated_bilinear__prompt_kernel(
    A_x: jax.Array,
    A_wqkv: jax.Array,
    A_wo: jax.Array,
    B_x: jax.Array,
    B_w_gate: jax.Array,
    B_w_up: jax.Array,
    B_w_down: jax.Array,
):
    return make()(A_x, A_wqkv, A_wo, B_x, B_w_gate, B_w_up, B_w_down)
```

```python
import functools

import jax
import jax.numpy as jnp
import jax.experimental.pallas as pl
import jax.experimental.pallas.tpu as pltpu

F32, BF16, U32 = jnp.float32, jnp.bfloat16, jnp.uint32
HEAD_DIM, WINDOW, DILATION, EPS = 32, 8, 2, 1e-5
LANES, PAD, GROUP = 128, 16, 16

LHS = ((0, 1, 3), (2, 1, 3), (0, 0, 0), (3, 0, 3), (0, 1, 1), (2, -1, 0), (1, -1, 3))
RHS = ((0, 1, 3), (0, 0, 0), (1, -1, 3), (2, -1, 0), (3, 0, 3), (0, 1, 1), (2, 1, 3))
ORDER = (1, 4, 0, 3, 2, 6, 5)
COMPLETES = {3: 2, 2: 1, 6: 0, 5: 3}


def _dot(a, b):
    return jnp.dot(a, b, preferred_element_type=F32)


def _comb(spec, get):
    i, sign, j = spec
    return get(i) if sign == 0 else get(i) + get(j) if sign > 0 else get(i) - get(j)


def _block(s, q):
    return s // 2 + q // 2 * 2, s % 2 + q % 2 * 2


class _Quadrants:
    def __init__(self, slots=None):
        self.slots = {} if slots is None else slots

    def add(self, o, m):
        t, done = self.slots, None
        if o == 1:
            t[0] = m
        elif o == 4:
            t[1] = m
        elif o == 0:
            t[4] = m
        elif o == 3:
            done = t[0] + m
            t[2] = m - t[1]
        elif o == 2:
            done = m + t[1]
            t[3] = m - t[0]
        else:
            done = t[2 if o == 6 else 3] + t[4] + m
        return done


def _two_levels(product, emit, slots):
    inner = _Quadrants(slots(0))
    outer = [_Quadrants(slots(s + 1)) for s in range(4)]
    for o in ORDER:
        for i in ORDER:
            v = inner.add(i, product(o, i))
            if v is not None:
                v = outer[COMPLETES[i]].add(o, v)
                if v is not None:
                    emit(COMPLETES[i], COMPLETES[o], v)


class _Parked:
    def __init__(self, refs, zero):
        self.refs, self.zero = refs, zero

    def __setitem__(self, k, v):
        self.shape = v.shape
        self.refs[k][:v.shape[0], :v.shape[1]] = v

    def __getitem__(self, k):
        return self.refs[k][pl.ds(pl.multiple_of(self.zero * 32, 32), self.shape[0]), :self.shape[1]]


def _identity(v):
    return v


class _SideWork:
    def __init__(self, jobs, first, last, never):
        self.jobs, self.slots, self.done, self.n, self.never = jobs, last - first + 1, 0, -first, never

    def step(self, product):
        self.n += 1
        end = min(len(self.jobs), -(-len(self.jobs) * self.n // self.slots))
        todo = self.jobs[self.done:max(end, self.done)]
        self.done += len(todo)
        rows = product.shape[0] // 8
        for k, job in enumerate(todo):
            col, row = divmod(k * rows * (product.shape[1] // LANES) // len(todo), rows)
            tile = product[8 * row:8 * row + 8, col * LANES:(col + 1) * LANES]

            def after(v, tile=tile):
                t = tile if v.dtype == F32 else pltpu.bitcast(tile, v.dtype)
                return jnp.where(self.never, jnp.concatenate([t] * (v.shape[0] // 8), axis=0), v)

            job(after)


def _rows(start, n):
    if isinstance(start, int):
        return pl.ds(start, n)
    index, step, offset = start
    return pl.ds(pl.multiple_of(index * step, step) + offset, n)


def _half(start):
    return start // 2 if isinstance(start, int) else (start[0], start[1] // 2, start[2] // 2)


def _put(ref, k, r0, cols, v):
    if ref.dtype == BF16:
        ref[k, _rows(r0, v.shape[0]), cols] = v.astype(BF16)
    else:
        ref[k, _rows(_half(r0), v.shape[0] // 2), cols] = pltpu.bitcast(v.astype(BF16), U32)


def _get(ref, k, r0, n, cols=slice(None)):
    if ref.dtype == BF16:
        return ref[k, _rows(r0, n), cols]
    return pltpu.bitcast(ref[k, _rows(_half(r0), n // 2), cols], BF16)


def _operand_buffer(n, rows, cols, words):
    return pltpu.VMEM((n, rows // 2, cols), U32) if words else pltpu.VMEM((n, rows, cols), BF16)


def _split_jobs(spec, load, store):
    blocks = []

    def job(o, after):
        quad = [after(_comb(spec[o], lambda q: blocks[_block(s, q)[0]][_block(s, q)[1]])) for s in range(4)]
        for i in range(7):
            store(7 * o + i, _comb(spec[i], quad.__getitem__))

    return [lambda after: blocks.extend(load(after))] + [functools.partial(job, o) for o in range(7)]


def _swap_block_lane(blocks):
    lane = jax.lax.broadcasted_iota(jnp.int32, blocks[0].shape, 1)
    t = [x if b == 0 else pltpu.roll(x, b, 1) for b, x in enumerate(blocks)]
    s = [t[(-c) % 8] for c in range(8)]
    for bit in (1, 2, 4):
        m = (lane & bit) != 0
        s = [jnp.where(m, s[(c - bit) % 8], s[c]) for c in range(8)]
    return [x if c == 0 else pltpu.roll(x, LANES - c, 1) for c, x in enumerate(s)]


def _attention(qkv, row, n):
    lane = jax.lax.broadcasted_iota(jnp.int32, (n, LANES), 1)
    pos = jax.lax.broadcasted_iota(jnp.int32, (n, LANES), 0) + (row[0] * row[1] + row[2])
    rows = [_rows(row[:2] + (row[2] + PAD - DILATION * w,), n) for w in range(WINDOW)]
    q = [qkv[0, c, rows[0], :] for c in range(8)]
    logits = []
    for w in range(WINDOW):
        s = functools.reduce(jnp.add, (q[c] * qkv[1, c, rows[w], :] for c in range(8)))
        s = s + pltpu.roll(s, LANES - 8, 1)
        s = s + pltpu.roll(s, LANES - 16, 1)
        s = s * (HEAD_DIM ** -0.5)
        logits.append(jnp.where(pos >= DILATION * w, s, -1e9) if w else s)
    m = functools.reduce(jnp.maximum, logits)
    e = [jnp.exp(s - m) for s in logits]
    inv = 1.0 / functools.reduce(jnp.add, e)
    p = []
    for w in range(WINDOW):
        a = e[w] * inv
        a = jnp.where((lane & 24) == 0, a, pltpu.roll(a, 8, 1))
        p.append(jnp.where((lane & 16) == 0, a, pltpu.roll(a, 16, 1)))
    return _swap_block_lane([
        functools.reduce(jnp.add, (p[w] * qkv[2, c, rows[w], :] for w in range(WINDOW)))
        for c in range(8)])


def _kernel(x_hbm, wqkv_hbm, wo_hbm, wg_hbm, wu_hbm, wd_hbm, out_hbm,
            x_v, wg_v, wu_v, wd_v, a2, wo2, acc, qkv, w_v, wp, a1, o2, tmp, hid, x_sem, w_sem, f_sem, o_sem, *, cfg):
    _, qm, d = x_hbm.shape
    tf = wg_v.shape[2]
    hd, qd, qf = d // 2, d // 4, tf // 4
    nf = wg_hbm.shape[1] // tf

    def f_copies(j, slot):
        c = pl.ds(pl.multiple_of(j * tf, tf), tf)
        return (pltpu.make_async_copy(wg_hbm.at[:, c], wg_v.at[slot], f_sem.at[0, slot]),
                pltpu.make_async_copy(wu_hbm.at[:, c], wu_v.at[slot], f_sem.at[1, slot]),
                pltpu.make_async_copy(wd_hbm.at[c, :], wd_v.at[slot], f_sem.at[2, slot]))

    def projections():
        br = qm // 4
        steps = cfg["steps"]
        xr, wr = br // steps, hd // steps

        def first_copies(g):
            r, k = (_rows(g * n if isinstance(g, int) else (g, n, 0), n) for n in (xr, wr))
            return (pltpu.make_async_copy(wqkv_hbm.at[:, k, pl.ds(0, d)], w_v.at[0, :, k], x_sem.at[1, g]),
                    pltpu.make_async_copy(x_hbm.at[:, r, :], x_v.at[:, r, :], x_sem.at[0, g]))

        def x_copy(g):
            r = _rows(g * br if isinstance(g, int) else (g, br, 0), br)
            return pltpu.make_async_copy(x_hbm.at[:, r, :], x_v.at[:, r, :], w_sem.at[2 + g])

        def w_copy(m):
            cols = pl.ds(pl.multiple_of(m * d, d), d)
            return pltpu.make_async_copy(wqkv_hbm.at[:, :, cols], w_v.at[m % 2], w_sem.at[m])

        wo_copy = pltpu.make_async_copy(wo_hbm, w_v.at[1], w_sem.at[0])

        def permuted_weight(m, i, r0, n, after=_identity):
            return _swap_block_lane([after(pltpu.bitcast(w_v[m, i, _rows(r0, n), c:c + LANES], U32))
                                     for c in range(0, d, LANES)])

        def normalized(q, r0, after=_identity):
            r = _rows(r0, GROUP)
            x = [after(x_v[q, r, c:c + LANES].astype(F32)) for c in range(0, d, LANES)]
            mean = jnp.sum(functools.reduce(jnp.add, x), axis=-1, keepdims=True) * (1.0 / d)
            x = [v - mean for v in x]
            var = jnp.sum(functools.reduce(jnp.add, [v * v for v in x]), axis=-1, keepdims=True) * (1.0 / d)
            rstd = jax.lax.rsqrt(var + EPS)
            hid[q][r, :] = jnp.broadcast_to(mean, (GROUP, LANES))
            hid[4 + q][r, :] = jnp.broadcast_to(rstd, (GROUP, LANES))
            return [v * rstd for v in x]

        def store_projection(m, q, r0, c0, v):
            n = v.shape[0] // 2
            for a in range(2):
                for p in range(0, v.shape[1], LANES):
                    qkv[m, c0 + (q % 2 * v.shape[1] + p) // LANES, _rows((r0[0], r0[1], r0[2] + PAD + (q // 2 * 2 + a) * qm), n), :] = (
                        v[a * n:(a + 1) * n, p:p + LANES])

        def one_level(m, r0, n, c0, rhs, work):
            c = _Quadrants()
            for o in ORDER:
                lhs = jnp.concatenate([a1[o][a, _rows(r0, n), :] for a in range(2)], axis=0)
                p = _dot(lhs, rhs(o))
                for s in work:
                    s.step(p)
                done = c.add(o, p)
                if done is not None:
                    store_projection(m, COMPLETES[o], r0, c0, done)

        for g in range(steps):
            for c in first_copies(g):
                c.start()
        x_copy(1).start()

        def first_body(g, carry):
            for c in first_copies(g):
                c.wait()
            w = [[pltpu.bitcast(v, BF16).astype(F32) for v in permuted_weight(0, i, (g, wr, 0), wr)] for i in range(2)]
            for p in range(4):
                for o in range(7):
                    _put(o2, 2 * o + p // 2, (g, wr, 0), slice(p % 2 * LANES, (p % 2 + 1) * LANES),
                         _comb(RHS[o], lambda q: w[q // 2][q % 2 * 4 + p]))
            for n in range(0, xr, GROUP):
                for a in range(2):
                    xn = [normalized(q, (g, xr, n)) for q in (a, a + 2)]
                    for p in range(4):
                        for o in range(7):
                            _put(a1[o], a, (g, xr, n), slice(p * LANES, (p + 1) * LANES),
                                 _comb(LHS[o], lambda q: xn[q // 2][q % 2 * 4 + p]))
            return carry

        jax.lax.fori_loop(0, steps, first_body, 0)

        def q_body(g, carry):
            @pl.when(g < 2)
            def _():
                x_copy(g + 2).start()

            pl.when(jnp.logical_or(g == 1, g == 2))(lambda: w_copy(g).start())
            pl.when(g == 3)(wo_copy.start)
            pl.when(g < 3)(lambda: x_copy(g + 1).wait())
            pl.when(g >= 2)(lambda: w_copy(g - 1).wait())
            nxt = (g + 1) % 4

            def permute(i, n, after):
                for c, v in enumerate(permuted_weight((g == 2).astype(jnp.int32), i, n, 32, after)):
                    wp[g // 3, (i * hd + n) // 2:(i * hd + n) // 2 + 16, c * LANES:(c + 1) * LANES] = v

            def normalize(n, a, after):
                for q in (a, a + 2):
                    for p, v in enumerate(normalized(q, (nxt, br, n), after)):
                        tmp[4 * q + p // 2][n:n + GROUP, p % 2 * LANES:(p % 2 + 1) * LANES] = v

            def operand(o, n, a, after):
                r = _rows((g // 4, 32, n), 32)
                for c in range(0, hd, LANES):
                    v = _comb(LHS[o], lambda q: tmp[4 * (a + q // 2 * 2) + q % 2 * 2 + c // qd][r, c % qd:c % qd + LANES])
                    _put(a1[o], a, (nxt, br, n), slice(c, c + LANES), after(v))

            never = g >= 4
            one_level(0, (g, br, 0), br, 0, lambda o: jnp.concatenate([_get(o2, 2 * o + b, 0, hd) for b in range(2)], axis=1), [
                _SideWork([functools.partial(normalize, n, a) for n in range(0, br, GROUP) for a in range(2)],
                          *cfg["norm"], never),
                _SideWork([functools.partial(permute, i, n) for i in range(2) for n in range(0, hd, 32)],
                          *cfg["perm"], never),
                _SideWork([functools.partial(operand, o, n, a) for o in ORDER for n in range(0, br, 32)
                           for a in range(2)], *cfg["opnd"], never)])
            return carry

        jax.lax.fori_loop(0, 4, q_body, 0)
        for c in f_copies(0, 0):
            c.start()
        wo_copy.wait()

        def weight_jobs(load, store, t, n):
            jobs = []
            for m in range(0, n, GROUP):
                for p in range(2):
                    jobs += _split_jobs(
                        RHS,
                        lambda after, m=m, p=p: [[after(load(i, (t, n, m), k, p).astype(F32))
                                                  for k in range(4)] for i in range(4)],
                        lambda k, v, m=m, p=p: store(k, (t, n, m), p, v))
            return jobs

        def wo_jobs(r0, n):
            return weight_jobs(lambda i, r, k, p: w_v[1, i // 2, _rows(r[:2] + (r[2] + i % 2 * qd,), GROUP),
                                                      p * hd + k * LANES:p * hd + (k + 1) * LANES],
                               lambda t, r, p, v: _put(wo2, 2 * t + p, r, slice(None), v), r0, n)

        def k_body(t, carry):
            def load(n, c, after):
                r = _rows((t, br, n), GROUP)
                mean = [after(hid[q][r, :]) for q in range(4)]
                return [[(x_v[q, r, k * qd + c:k * qd + c + LANES].astype(F32) - mean[q]) * hid[4 + q][r, :]
                         for k in range(4)] for q in range(4)]

            jobs = []
            for n in range(0, br, GROUP):
                for c in (0, LANES):
                    jobs += _split_jobs(LHS, functools.partial(load, n, c),
                                        lambda k, v, n=n, c=c: _put(a2, k, (t, br, n), slice(c, c + LANES), v))
            wv_jobs = weight_jobs(lambda i, r, k, p: _get(wp, 1, r[:2] + (r[2] + i * qd,), GROUP,
                                                          slice((2 * k + p) * LANES, (2 * k + p + 1) * LANES)),
                                  lambda k, r, p, v: _put(o2, k, r[:2] + (r[2] + p * qd,), slice(0, LANES), v),
                                  t, qd // 4)
            w = [_get(wp, 0, q // 2 * hd, hd, pl.ds(pl.multiple_of(t % 2 * hd, hd) + q % 2 * qd, qd)).astype(F32)
                 for q in range(4)]
            one_level(1, (t // 2, qm // 2, 0), qm // 2, t % 2 * 4, lambda o: _comb(RHS[o], w.__getitem__).astype(BF16),
                      [_SideWork(jobs, *cfg["a2"], t >= 4), _SideWork(wv_jobs, *cfg["wv"], t >= 4)])
            return carry

        jax.lax.fori_loop(0, 4, k_body, 0)

        nv = cfg["nv"]
        vr = qm // nv

        def v_body(t, carry):
            def clear(k, after):
                zero = after(jnp.zeros((8, LANES), F32))
                acc[k, t % 2, _rows((t // 2, vr, 0), vr), :] = jnp.tile(zero, (vr // 8, 1))

            never = t >= 2 * nv
            work = [_SideWork([functools.partial(clear, k) for k in range(49)], *cfg["zero"], never),
                    _SideWork(wo_jobs(t, qd // (2 * nv)), *cfg["wo"], never)]

            def product(o, i):
                p = _dot(_get(a2, 7 * o + i, (t // 2, vr, 0), vr), _get(o2, 7 * o + i, (t % 2, qd, 0), qd, slice(0, LANES)))
                for s in work:
                    s.step(p)
                return p

            def emit(s, q, v):
                i, k = _block(s, q)
                qkv[2, 2 * k + t % 2, _rows((t // 2, vr, PAD + i * qm), vr), :] = v

            _two_levels(product, emit, lambda s: None)
            return carry

        jax.lax.fori_loop(0, 2 * nv, v_body, 0, unroll=cfg["vu"])

    projections()

    for m in (1, 2):
        for c in range(8):
            qkv[m, c, :PAD, :] = jnp.broadcast_to(qkv[m, c, PAD:PAD + 1, :], (PAD, LANES))

    def rest():
        groups = -(-qm // (GROUP * nf))

        def ffn_body(j, carry):
            slot = j % 2

            @pl.when(j + 1 < nf)
            def _():
                for c in f_copies(j + 1, 1 - slot):
                    c.start()

            for c in f_copies(j, slot):
                c.wait()

            att, jobs = [], []
            for n in range(groups):
                r0 = (j, (groups - 1) * GROUP, n * GROUP)
                if n == groups - 1:
                    r0 = (jnp.where(j < qm // GROUP - nf * (groups - 1), j, 0), GROUP, nf * (groups - 1) * GROUP)
                att.append([_attention(qkv, r0[:2] + (r0[2] + q * qm,), GROUP) for q in range(4)])
                for p in range(2):
                    jobs += _split_jobs(
                        LHS, lambda after, n=n, p=p: [[att[n][q][2 * k + p] for k in range(4)] for q in range(4)],
                        lambda t, v, r0=r0, p=p: _put(o2, t, r0, slice(p * LANES, (p + 1) * LANES), v))
            if cfg["att"] is None:
                for job in jobs:
                    job(_identity)
                jobs = []
            work = _SideWork(jobs, *(cfg["att"] or (0, 1)), j >= nf)

            def w_in(s, q):
                i, k = _block(s, q)
                r, c = slice(i * qd, (i + 1) * qd), slice(k * qf, (k + 1) * qf)
                return jnp.concatenate([wg_v[slot, r, c].astype(F32), wu_v[slot, r, c].astype(F32)], axis=1)

            def w_out(s, q):
                i, k = _block(s, q)
                return jnp.concatenate([wd_v[slot, i * qf:(i + 1) * qf, c + k * LANES:c + (k + 1) * LANES].astype(F32)
                                        for c in (0, hd)], axis=1)

            def operand(spec, o, i, get):
                return _comb(spec[i], lambda s: _comb(spec[o], lambda q: get(s, q))).astype(BF16)

            h = _Parked(hid, j // nf)

            def gate(s, q, v):
                h[4 * s + q] = v[:, :qf] * v[:, qf:]

            def product(o, i):
                p = _dot(_get(a2, 7 * o + i, 0, qm), operand(RHS, o, i, w_in))
                work.step(p)
                return p

            _two_levels(product, gate, lambda s: _Parked(tmp[5 * s:], j // nf))
            for o in cfg["down"][0]:
                for i in cfg["down"][1]:
                    p = _dot(operand(LHS, o, i, lambda s, q: h[4 * s + q]), operand(RHS, o, i, w_out))
                    for c in range(2):
                        acc[7 * o + i, c] += p[:, c * LANES:(c + 1) * LANES]
                    work.step(p)
            return carry

        if not cfg["skip"]:
            jax.lax.fori_loop(0, nf, ffn_body, 0)

        no = cfg["no"]
        rows = qm // no

        def o_copy(t):
            at = (slice(None), _rows(t // 2 * rows if isinstance(t, int) else (t // 2, rows, 0), rows), pl.ds(pl.multiple_of(t % 2 * hd, hd), hd))
            return pltpu.make_async_copy(x_v.at[at], out_hbm.at[at], o_sem.at[t])

        def out_body(t, carry):
            r = _rows(t // 2 * rows if isinstance(t, int) else (t // 2, rows, 0), rows)

            def product(o, i):
                p = _dot(_get(o2, 7 * o + i, (t // 2, rows, 0), rows), _get(wo2, 2 * (7 * o + i) + t % 2, 0, qd))
                return p + acc[7 * o + i, t % 2, r, :]

            def emit(s, q, v):
                i, k = _block(s, q)
                at = (i, r, pl.ds(pl.multiple_of(t % 2 * hd, hd) + k * LANES, LANES))
                x_v[at] = (x_v[at].astype(F32) + v).astype(BF16)

            _two_levels(product, emit,
                        lambda s: _Parked(tmp[5 * s:], t // (2 * no)) if s in cfg["opark"] else None)
            o_copy(t).start()
            return carry

        jax.lax.fori_loop(0, 2 * no, out_body, 0)
        for t in range(2 * no):
            o_copy(t).wait()

    rest()


CONFIG = dict(steps=4, norm=(0, 3), perm=(0, 5), opnd=(5, 6), a2=(0, 3), wv=(4, 5), nv=4, zero=(20, 44), wo=(0, 30),
              words="lo", down=((2, 4, 5, 3, 1, 6, 0), (3, 2, 4, 5, 1, 6, 0)), skip=False, no=4, opark=(), att=(18, 96), vu=1)


def make(flags={"XLA_TPU_EVENLY_DISTRIBUTE_CRITICAL_NODES": True}, **overrides):
    cfg = dict(CONFIG, **overrides)

    def fn(A_x, A_wqkv, A_wo, B_x, B_w_gate, B_w_up, B_w_down):
        del B_x
        b, s, d = A_x.shape
        qm, tf = s // 4, 4 * LANES
        any_spec = pl.BlockSpec(memory_space=pl.ANY)
        out = pl.pallas_call(
            functools.partial(_kernel, cfg=cfg),
            in_specs=[any_spec] * 6,
            out_specs=any_spec,
            out_shape=jax.ShapeDtypeStruct((4, qm, d), A_x.dtype),
            scratch_shapes=[
                pltpu.VMEM((4, qm, d), BF16),
                pltpu.VMEM((2, d, tf), BF16),
                pltpu.VMEM((2, d, tf), BF16),
                pltpu.VMEM((2, tf, d), BF16),
                _operand_buffer(49, qm, d // 4, True),
                _operand_buffer(98, d // 4, LANES, "o" in cfg["words"]),
                pltpu.VMEM((49, 2, qm, LANES), F32),
                pltpu.VMEM((3, 8, PAD + s, LANES), F32),
                pltpu.VMEM((2, 2, d // 2, d), BF16),
                pltpu.VMEM((2, d // 2, d), U32),
                [pltpu.VMEM((2, qm, d // 2), BF16)] * 7,
                _operand_buffer(49, qm, d // 4, "l" in cfg["words"]),
                [pltpu.VMEM((qm, tf // 2), F32)] * 25,
                [pltpu.VMEM((qm, tf // 4), F32)] * 16,
                pltpu.SemaphoreType.DMA((2, cfg["steps"])),
                pltpu.SemaphoreType.DMA((6,)),
                pltpu.SemaphoreType.DMA((3, 2)),
                pltpu.SemaphoreType.DMA((2 * cfg["no"],)),
            ],
            compiler_params=pltpu.CompilerParams(vmem_limit_bytes=126 * 2 ** 20, flags=flags,
                                                 disable_bounds_checks=True),
        )(A_x.reshape(4, qm, d), A_wqkv.reshape(2, d // 2, 3 * d), A_wo.reshape(2, d // 2, d), B_w_gate, B_w_up, B_w_down)
        return out.reshape(b, s, d)
    return fn


@jax.jit
def pallas_parallel_sum__sliding_local_dilated__glu_gated_bilinear__prompt_kernel(
    A_x: jax.Array,
    A_wqkv: jax.Array,
    A_wo: jax.Array,
    B_x: jax.Array,
    B_w_gate: jax.Array,
    B_w_up: jax.Array,
    B_w_down: jax.Array,
):
    return make()(A_x, A_wqkv, A_wo, B_x, B_w_gate, B_w_up, B_w_down)
```

```python
import functools

import jax
import jax.numpy as jnp
import jax.experimental.pallas as pl
import jax.experimental.pallas.tpu as pltpu

F32, BF16, U32 = jnp.float32, jnp.bfloat16, jnp.uint32
HEAD_DIM, WINDOW, DILATION, EPS = 32, 8, 2, 1e-5
LANES, PAD, GROUP = 128, 16, 16

LHS = ((0, 1, 3), (2, 1, 3), (0, 0, 0), (3, 0, 3), (0, 1, 1), (2, -1, 0), (1, -1, 3))
RHS = ((0, 1, 3), (0, 0, 0), (1, -1, 3), (2, -1, 0), (3, 0, 3), (0, 1, 1), (2, 1, 3))
ORDER = (1, 4, 0, 3, 2, 6, 5)
COMPLETES = {3: 2, 2: 1, 6: 0, 5: 3}


def _dot(a, b):
    return jnp.dot(a, b, preferred_element_type=F32)


def _comb(spec, get):
    i, sign, j = spec
    return get(i) if sign == 0 else get(i) + get(j) if sign > 0 else get(i) - get(j)


def _block(s, q):
    return s // 2 + q // 2 * 2, s % 2 + q % 2 * 2


class _Quadrants:
    def __init__(self, slots=None):
        self.slots = {} if slots is None else slots

    def add(self, o, m):
        t, done = self.slots, None
        if o == 1:
            t[0] = m
        elif o == 4:
            t[1] = m
        elif o == 0:
            t[4] = m
        elif o == 3:
            done = t[0] + m
            t[2] = m - t[1]
        elif o == 2:
            done = m + t[1]
            t[3] = m - t[0]
        else:
            done = t[2 if o == 6 else 3] + t[4] + m
        return done


def _two_levels(product, emit, slots):
    inner = _Quadrants(slots(0))
    outer = [_Quadrants(slots(s + 1)) for s in range(4)]
    for o in ORDER:
        for i in ORDER:
            v = inner.add(i, product(o, i))
            if v is not None:
                v = outer[COMPLETES[i]].add(o, v)
                if v is not None:
                    emit(COMPLETES[i], COMPLETES[o], v)


class _Parked:
    def __init__(self, refs, zero):
        self.refs, self.zero = refs, zero

    def __setitem__(self, k, v):
        self.shape = v.shape
        self.refs[k][:v.shape[0], :v.shape[1]] = v

    def __getitem__(self, k):
        return self.refs[k][pl.ds(pl.multiple_of(self.zero * 32, 32), self.shape[0]), :self.shape[1]]


def _identity(v):
    return v


class _SideWork:
    def __init__(self, jobs, first, last, never):
        self.jobs, self.slots, self.done, self.n, self.never = jobs, last - first + 1, 0, -first, never

    def step(self, product):
        self.n += 1
        end = min(len(self.jobs), -(-len(self.jobs) * self.n // self.slots))
        todo = self.jobs[self.done:max(end, self.done)]
        self.done += len(todo)
        rows = product.shape[0] // 8
        for k, job in enumerate(todo):
            col, row = divmod(k * rows * (product.shape[1] // LANES) // len(todo), rows)
            tile = product[8 * row:8 * row + 8, col * LANES:(col + 1) * LANES]

            def after(v, tile=tile):
                t = tile if v.dtype == F32 else pltpu.bitcast(tile, v.dtype)
                return jnp.where(self.never, jnp.concatenate([t] * (v.shape[0] // 8), axis=0), v)

            job(after)


def _rows(start, n):
    if isinstance(start, int):
        return pl.ds(start, n)
    index, step, offset = start
    return pl.ds(pl.multiple_of(index * step, step) + offset, n)


def _half(start):
    return start // 2 if isinstance(start, int) else (start[0], start[1] // 2, start[2] // 2)


def _put(ref, k, r0, cols, v):
    if ref.dtype == BF16:
        ref[k, _rows(r0, v.shape[0]), cols] = v.astype(BF16)
    else:
        ref[k, _rows(_half(r0), v.shape[0] // 2), cols] = pltpu.bitcast(v.astype(BF16), U32)


def _get(ref, k, r0, n, cols=slice(None)):
    if ref.dtype == BF16:
        return ref[k, _rows(r0, n), cols]
    return pltpu.bitcast(ref[k, _rows(_half(r0), n // 2), cols], BF16)


def _operand_buffer(n, rows, cols, words):
    return pltpu.VMEM((n, rows // 2, cols), U32) if words else pltpu.VMEM((n, rows, cols), BF16)


def _split_jobs(spec, load, store):
    blocks = []

    def job(o, after):
        quad = [after(_comb(spec[o], lambda q: blocks[_block(s, q)[0]][_block(s, q)[1]])) for s in range(4)]
        for i in range(7):
            store(7 * o + i, _comb(spec[i], quad.__getitem__))

    return [lambda after: blocks.extend(load(after))] + [functools.partial(job, o) for o in range(7)]


def _swap_block_lane(blocks):
    lane = jax.lax.broadcasted_iota(jnp.int32, blocks[0].shape, 1)
    t = [x if b == 0 else pltpu.roll(x, b, 1) for b, x in enumerate(blocks)]
    s = [t[(-c) % 8] for c in range(8)]
    for bit in (1, 2, 4):
        m = (lane & bit) != 0
        s = [jnp.where(m, s[(c - bit) % 8], s[c]) for c in range(8)]
    return [x if c == 0 else pltpu.roll(x, LANES - c, 1) for c, x in enumerate(s)]


def _attention(qkv, row, n, out):
    rows = [_rows(row[:2] + (row[2] + PAD - DILATION * w,), n) for w in range(WINDOW)]
    logits, p = [], []

    def scores(after):
        pos = jax.lax.broadcasted_iota(jnp.int32, (n, LANES), 0) + (row[0] * row[1] + row[2])
        q = [after(qkv[0, c, rows[0], :]) for c in range(8)]
        for w in range(WINDOW):
            s = functools.reduce(jnp.add, (q[c] * qkv[1, c, rows[w], :] for c in range(8)))
            s = s + pltpu.roll(s, LANES - 8, 1)
            s = s + pltpu.roll(s, LANES - 16, 1)
            s = s * (HEAD_DIM ** -0.5)
            logits.append(jnp.where(pos >= DILATION * w, s, -1e9) if row[2] < DILATION * w else s)

    def softmax(after):
        lane = jax.lax.broadcasted_iota(jnp.int32, (n, LANES), 1)
        m = after(functools.reduce(jnp.maximum, logits))
        e = [jnp.exp(s - m) for s in logits]
        inv = 1.0 / functools.reduce(jnp.add, e)
        for w in range(WINDOW):
            a = e[w] * inv
            a = jnp.where((lane & 24) == 0, a, pltpu.roll(a, 8, 1))
            p.append(jnp.where((lane & 16) == 0, a, pltpu.roll(a, 16, 1)))

    def values(after):
        p[0] = after(p[0])
        out.extend(_swap_block_lane([
            functools.reduce(jnp.add, (p[w] * qkv[2, c, rows[w], :] for w in range(WINDOW))) for c in range(8)]))

    return scores, softmax, values


def _kernel(x_hbm, wqkv_hbm, wo_hbm, wg_hbm, wu_hbm, wd_hbm, out_hbm,
            x_v, wg_v, wu_v, wd_v, a2, wo2, acc, qkv, w_v, wp, a1, o2, tmp, hid, x_sem, w_sem, f_sem, o_sem, *, cfg):
    _, qm, d = x_hbm.shape
    tf = wg_v.shape[2]
    hd, qd, qf = d // 2, d // 4, tf // 4
    nf = wg_hbm.shape[1] // tf

    def f_copies(j, slot):
        c = pl.ds(pl.multiple_of(j * tf, tf), tf)
        return (pltpu.make_async_copy(wg_hbm.at[:, c], wg_v.at[slot], f_sem.at[0, slot]),
                pltpu.make_async_copy(wu_hbm.at[:, c], wu_v.at[slot], f_sem.at[1, slot]),
                pltpu.make_async_copy(wd_hbm.at[c, :], wd_v.at[slot], f_sem.at[2, slot]))

    def projections():
        br = qm // 4
        steps, pn = cfg["steps"], cfg["pn"]
        xr, wr = br // steps, hd // steps

        def first_copies(g):
            r, k = (_rows(g * n if isinstance(g, int) else (g, n, 0), n) for n in (xr, wr))
            return (pltpu.make_async_copy(wqkv_hbm.at[:, k, pl.ds(0, d)], w_v.at[0, :, k], x_sem.at[1, g]),
                    pltpu.make_async_copy(x_hbm.at[:, r, :], x_v.at[:, r, :], x_sem.at[0, g]))

        def x_copy(g):
            r = _rows(g * br if isinstance(g, int) else (g, br, 0), br)
            return pltpu.make_async_copy(x_hbm.at[:, r, :], x_v.at[:, r, :], w_sem.at[2 + g])

        def w_copy(m):
            cols = pl.ds(pl.multiple_of(m * d, d), d)
            return pltpu.make_async_copy(wqkv_hbm.at[:, :, cols], w_v.at[m % 2], w_sem.at[m])

        wo_copy = pltpu.make_async_copy(wo_hbm, w_v.at[1], w_sem.at[0])

        def permuted_weight(m, i, r0, n, after=_identity):
            return _swap_block_lane([after(pltpu.bitcast(w_v[m, i, _rows(r0, n), c:c + LANES], U32))
                                     for c in range(0, d, LANES)])

        def normalized(q, r0, after=_identity):
            r = _rows(r0, GROUP)
            x = [after(x_v[q, r, c:c + LANES].astype(F32)) for c in range(0, d, LANES)]
            mean = jnp.sum(functools.reduce(jnp.add, x), axis=-1, keepdims=True) * (1.0 / d)
            x = [v - mean for v in x]
            var = jnp.sum(functools.reduce(jnp.add, [v * v for v in x]), axis=-1, keepdims=True) * (1.0 / d)
            rstd = jax.lax.rsqrt(var + EPS)
            hid[q][r, :] = jnp.broadcast_to(mean, (GROUP, LANES))
            hid[4 + q][r, :] = jnp.broadcast_to(rstd, (GROUP, LANES))
            return [v * rstd for v in x]

        def store_projection(m, q, r0, c0, v):
            n = v.shape[0] // 2
            for a in range(2):
                for p in range(0, v.shape[1], LANES):
                    qkv[m, c0 + (q % 2 * v.shape[1] + p) // LANES, _rows((r0[0], r0[1], r0[2] + PAD + (q // 2 * 2 + a) * qm), n), :] = (
                        v[a * n:(a + 1) * n, p:p + LANES])

        def one_level(m, r0, n, c0, rhs, work):
            c = _Quadrants()
            for o in ORDER:
                lhs = jnp.concatenate([_get(a1[o], a, r0, n) for a in range(2)], axis=0)
                p = _dot(lhs, rhs(o))
                for s in work:
                    s.step(p)
                done = c.add(o, p)
                if done is not None:
                    store_projection(m, COMPLETES[o], r0, c0, done)

        for g in range(steps):
            for c in first_copies(g):
                c.start()
        x_copy(1).start()

        def first_body(g, carry):
            for c in first_copies(g):
                c.wait()
            w = [[pltpu.bitcast(v, BF16).astype(F32) for v in permuted_weight(0, i, (g, wr, 0), wr)] for i in range(2)]
            for p in range(4):
                for o in range(7):
                    _put(o2, 2 * o + p // 2, (g, wr, 0), slice(p % 2 * LANES, (p % 2 + 1) * LANES),
                         _comb(RHS[o], lambda q: w[q // 2][q % 2 * 4 + p]))
            for n in range(0, xr, GROUP):
                for a in range(2):
                    xn = [normalized(q, (g, xr, n)) for q in (a, a + 2)]
                    for p in range(4):
                        for o in range(7):
                            _put(a1[o], a, (g, xr, n), slice(p * LANES, (p + 1) * LANES),
                                 _comb(LHS[o], lambda q: xn[q // 2][q % 2 * 4 + p]))
            return carry

        jax.lax.fori_loop(0, steps, first_body, 0)

        def q_body(g, carry):
            @pl.when(g < 2)
            def _():
                x_copy(g + 2).start()

            pl.when(jnp.logical_or(g == 1, g == 2))(lambda: w_copy(g).start())
            pl.when(g == 3)(wo_copy.start)
            pl.when(g < 3)(lambda: x_copy(g + 1).wait())
            pl.when(g >= 2)(lambda: w_copy(g - 1).wait())
            nxt = (g + 1) % 4

            def permute(i, n, after):
                for c, v in enumerate(permuted_weight((g == 2).astype(jnp.int32), i, n, pn, after)):
                    wp[g // 3, (i * hd + n) // 2:(i * hd + n + pn) // 2, c * LANES:(c + 1) * LANES] = v

            def normalize(n, a, after):
                for q in (a, a + 2):
                    for p, v in enumerate(normalized(q, (nxt, br, n), after)):
                        tmp[4 * q + p // 2][n:n + GROUP, p % 2 * LANES:(p % 2 + 1) * LANES] = v

            def operand(o, n, a, after):
                r = _rows((g // 4, 32, n), 32)
                for c in range(0, hd, LANES):
                    v = _comb(LHS[o], lambda q: tmp[4 * (a + q // 2 * 2) + q % 2 * 2 + c // qd][r, c % qd:c % qd + LANES])
                    _put(a1[o], a, (nxt, br, n), slice(c, c + LANES), after(v))

            never = g >= 4
            one_level(0, (g, br, 0), br, 0, lambda o: jnp.concatenate([_get(o2, 2 * o + b, 0, hd) for b in range(2)], axis=1), [
                _SideWork([functools.partial(normalize, n, a) for n in range(0, br, GROUP) for a in range(2)],
                          *cfg["norm"], never),
                _SideWork([functools.partial(permute, i, n) for i in range(2) for n in range(0, hd, pn)],
                          *cfg["perm"], never),
                _SideWork([functools.partial(operand, o, n, a) for o in ORDER for n in range(0, br, 32)
                           for a in range(2)], *cfg["opnd"], never)])
            return carry

        jax.lax.fori_loop(0, 4, q_body, 0)
        for c in f_copies(0, 0):
            c.start()
        wo_copy.wait()

        def weight_jobs(load, store, t, n):
            jobs = []
            for m in range(0, n, GROUP):
                for p in range(2):
                    jobs += _split_jobs(
                        RHS,
                        lambda after, m=m, p=p: [[after(load(i, (t, n, m), k, p).astype(F32))
                                                  for k in range(4)] for i in range(4)],
                        lambda k, v, m=m, p=p: store(k, (t, n, m), p, v))
            return jobs

        def wo_jobs(r0, n):
            return weight_jobs(lambda i, r, k, p: w_v[1, i // 2, _rows(r[:2] + (r[2] + i % 2 * qd,), GROUP),
                                                      p * hd + k * LANES:p * hd + (k + 1) * LANES],
                               lambda t, r, p, v: _put(wo2, 2 * t + p, r, slice(None), v), r0, n)

        def k_body(t, carry):
            def load(n, c, after):
                r = _rows((t, br, n), GROUP)
                mean = [after(hid[q][r, :]) for q in range(4)]
                return [[(x_v[q, r, k * qd + c:k * qd + c + LANES].astype(F32) - mean[q]) * hid[4 + q][r, :]
                         for k in range(4)] for q in range(4)]

            jobs = []
            for n in range(0, br, GROUP):
                for c in (0, LANES):
                    jobs += _split_jobs(LHS, functools.partial(load, n, c),
                                        lambda k, v, n=n, c=c: _put(a2, k, (t, br, n), slice(c, c + LANES), v))
            wv_jobs = weight_jobs(lambda i, r, k, p: _get(wp, 1, r[:2] + (r[2] + i * qd,), GROUP,
                                                          slice((2 * k + p) * LANES, (2 * k + p + 1) * LANES)),
                                  lambda k, r, p, v: _put(o2, k, r[:2] + (r[2] + p * qd,), slice(0, LANES), v),
                                  t, qd // 4)
            w = [_get(wp, 0, q // 2 * hd, hd, pl.ds(pl.multiple_of(t % 2 * hd, hd) + q % 2 * qd, qd)).astype(F32)
                 for q in range(4)]
            one_level(1, (t // 2, qm // 2, 0), qm // 2, t % 2 * 4, lambda o: _comb(RHS[o], w.__getitem__).astype(BF16),
                      [_SideWork(jobs, *cfg["a2"], t >= 4), _SideWork(wv_jobs, *cfg["wv"], t >= 4)])
            return carry

        jax.lax.fori_loop(0, 4, k_body, 0)

        nv = cfg["nv"]
        vr = qm // nv

        def v_body(t, carry):
            def clear(k, after):
                zero = after(jnp.zeros((8, LANES), F32))
                acc[k, t % 2, _rows((t // 2, vr, 0), vr), :] = jnp.tile(zero, (vr // 8, 1))

            never = t >= 2 * nv
            work = [_SideWork([functools.partial(clear, k) for k in range(49)], *cfg["zero"], never),
                    _SideWork(wo_jobs(t, qd // (2 * nv)), *cfg["wo"], never)]

            def product(o, i):
                p = _dot(_get(a2, 7 * o + i, (t // 2, vr, 0), vr), _get(o2, 7 * o + i, (t % 2, qd, 0), qd, slice(0, LANES)))
                for s in work:
                    s.step(p)
                return p

            def emit(s, q, v):
                i, k = _block(s, q)
                qkv[2, 2 * k + t % 2, _rows((t // 2, vr, PAD + i * qm), vr), :] = v

            _two_levels(product, emit, lambda s: None)
            return carry

        jax.lax.fori_loop(0, 2 * nv, v_body, 0, unroll=cfg["vu"])

    projections()

    for m in (1, 2):
        for c in range(8):
            qkv[m, c, :PAD, :] = jnp.broadcast_to(qkv[m, c, PAD:PAD + 1, :], (PAD, LANES))

    def rest():
        groups = -(-qm // (GROUP * nf))

        def ffn_body(j, carry):
            slot = j % 2

            @pl.when(j + 1 < nf)
            def _():
                for c in f_copies(j + 1, 1 - slot):
                    c.start()

            for c in f_copies(j, slot):
                c.wait()

            att, units, jobs = [], [], []
            for n in range(groups if cfg["au"] else 0):
                r0 = (j, (groups - 1) * GROUP, n * GROUP)
                if n == groups - 1:
                    r0 = (jnp.where(j < qm // GROUP - nf * (groups - 1), j, 0), GROUP, nf * (groups - 1) * GROUP)
                an = cfg["an"]
                att.append([[[] for _ in range(0, GROUP, an)] for q in range(4)])
                units += [_attention(qkv, r0[:2] + (r0[2] + q * qm + k,), an, att[n][q][k // an])
                          for q in range(4) for k in range(0, GROUP, an)]
                for p in range(2):
                    jobs += _split_jobs(
                        LHS, lambda after, n=n, p=p: [[jnp.concatenate([v[2 * k + p] for v in att[n][q]], axis=0) for k in range(4)] for q in range(4)],
                        lambda t, v, r0=r0, p=p: _put(o2, t, r0, slice(p * LANES, (p + 1) * LANES), v))
            lag = cfg["lag"]
            stages = [units[u - lag[k]][k] for u in range(len(units) + lag[2]) for k in cfg["so"]
                      if 0 <= u - lag[k] < len(units)]
            if cfg["pace"] is None:
                for job in stages:
                    job(_identity)
                stages = []
            work = _SideWork(jobs, *cfg["att"], j >= nf)
            early = _SideWork(stages, *(cfg["pace"] or (0, 1)), j >= nf)

            def w_in(s, q):
                i, k = _block(s, q)
                r, c = slice(i * qd, (i + 1) * qd), slice(k * qf, (k + 1) * qf)
                return jnp.concatenate([wg_v[slot, r, c].astype(F32), wu_v[slot, r, c].astype(F32)], axis=1)

            def w_out(s, q):
                i, k = _block(s, q)
                return jnp.concatenate([wd_v[slot, i * qf:(i + 1) * qf, c + k * LANES:c + (k + 1) * LANES].astype(F32)
                                        for c in (0, hd)], axis=1)

            def operand(spec, o, i, get):
                return _comb(spec[i], lambda s: _comb(spec[o], lambda q: get(s, q))).astype(BF16)

            h = _Parked(hid, j // nf)

            def gate(s, q, v):
                h[4 * s + q] = v[:, :qf] * v[:, qf:]

            def product(o, i):
                p = _dot(_get(a2, 7 * o + i, 0, qm), operand(RHS, o, i, w_in))
                early.step(p)
                work.step(p)
                return p

            _two_levels(product, gate, lambda s: _Parked(tmp[5 * s:], j // nf) if s in cfg["fpark"] else None)
            for o in cfg["down"][0]:
                for i in cfg["down"][1]:
                    p = _dot(operand(LHS, o, i, lambda s, q: h[4 * s + q]), operand(RHS, o, i, w_out))
                    for c in range(2):
                        acc[7 * o + i, c] += p[:, c * LANES:(c + 1) * LANES]
                    early.step(p)
                    work.step(p)
            return carry

        if not cfg["skip"]:
            jax.lax.fori_loop(0, nf, ffn_body, 0)

        no = cfg["no"]
        rows = qm // no

        def o_copy(t):
            at = (slice(None), _rows(t // 2 * rows if isinstance(t, int) else (t // 2, rows, 0), rows), pl.ds(pl.multiple_of(t % 2 * hd, hd), hd))
            return pltpu.make_async_copy(x_v.at[at], out_hbm.at[at], o_sem.at[t])

        def out_body(t, carry):
            r = _rows(t // 2 * rows if isinstance(t, int) else (t // 2, rows, 0), rows)

            def product(o, i):
                p = _dot(_get(o2, 7 * o + i, (t // 2, rows, 0), rows), _get(wo2, 2 * (7 * o + i) + t % 2, 0, qd))
                return p + acc[7 * o + i, t % 2, r, :]

            def emit(s, q, v):
                i, k = _block(s, q)
                at = (i, r, pl.ds(pl.multiple_of(t % 2 * hd, hd) + k * LANES, LANES))
                x_v[at] = (x_v[at].astype(F32) + v).astype(BF16)

            _two_levels(product, emit,
                        lambda s: _Parked(tmp[5 * s:], t // (2 * no)) if s in cfg["opark"] else None)
            o_copy(t).start()
            return carry

        jax.lax.fori_loop(0, 2 * no, out_body, 0)
        for t in range(2 * no):
            o_copy(t).wait()

    rest()


CONFIG = dict(steps=4, norm=(0, 2), perm=(1, 4), opnd=(4, 6), a2=(0, 4), wv=(4, 6), nv=4, zero=(20, 44), wo=(0, 30),
              words="loa", down=((2, 4, 5, 3, 1, 6, 0), (3, 2, 4, 5, 1, 6, 0)), skip=False, no=4, opark=(), att=(18, 96), vu=1, an=16, lag=(0, 2, 2), so=(0, 1, 2), pace=None, au=1, fpark=(0, 1, 2, 3, 4), pn=16)


def make(flags={"XLA_TPU_EVENLY_DISTRIBUTE_CRITICAL_NODES": True}, **overrides):
    cfg = dict(CONFIG, **overrides)

    def fn(A_x, A_wqkv, A_wo, B_x, B_w_gate, B_w_up, B_w_down):
        del B_x
        b, s, d = A_x.shape
        qm, tf = s // 4, 4 * LANES
        any_spec = pl.BlockSpec(memory_space=pl.ANY)
        out = pl.pallas_call(
            functools.partial(_kernel, cfg=cfg),
            in_specs=[any_spec] * 6,
            out_specs=any_spec,
            out_shape=jax.ShapeDtypeStruct((4, qm, d), A_x.dtype),
            scratch_shapes=[
                pltpu.VMEM((4, qm, d), BF16),
                pltpu.VMEM((2, d, tf), BF16),
                pltpu.VMEM((2, d, tf), BF16),
                pltpu.VMEM((2, tf, d), BF16),
                _operand_buffer(49, qm, d // 4, True),
                _operand_buffer(98, d // 4, LANES, "o" in cfg["words"]),
                pltpu.VMEM((49, 2, qm, LANES), F32),
                pltpu.VMEM((3, 8, PAD + s, LANES), F32),
                pltpu.VMEM((2, 2, d // 2, d), BF16),
                pltpu.VMEM((2, d // 2, d), U32),
                [_operand_buffer(2, qm, d // 2, "a" in cfg["words"])] * 7,
                _operand_buffer(49, qm, d // 4, "l" in cfg["words"]),
                [pltpu.VMEM((qm, tf // 2), F32)] * 25,
                [pltpu.VMEM((qm, tf // 4), F32)] * 16,
                pltpu.SemaphoreType.DMA((2, cfg["steps"])),
                pltpu.SemaphoreType.DMA((6,)),
                pltpu.SemaphoreType.DMA((3, 2)),
                pltpu.SemaphoreType.DMA((2 * cfg["no"],)),
            ],
            compiler_params=pltpu.CompilerParams(vmem_limit_bytes=126 * 2 ** 20, flags=flags,
                                                 disable_bounds_checks=True),
        )(A_x.reshape(4, qm, d), A_wqkv.reshape(2, d // 2, 3 * d), A_wo.reshape(2, d // 2, d), B_w_gate, B_w_up, B_w_down)
        return out.reshape(b, s, d)
    return fn


@jax.jit
def pallas_parallel_sum__sliding_local_dilated__glu_gated_bilinear__prompt_kernel(
    A_x: jax.Array,
    A_wqkv: jax.Array,
    A_wo: jax.Array,
    B_x: jax.Array,
    B_w_gate: jax.Array,
    B_w_up: jax.Array,
    B_w_down: jax.Array,
):
    return make()(A_x, A_wqkv, A_wo, B_x, B_w_gate, B_w_up, B_w_down)
```

```python
import functools

import jax
import jax.numpy as jnp
import jax.experimental.pallas as pl
import jax.experimental.pallas.tpu as pltpu

F32, BF16, U32 = jnp.float32, jnp.bfloat16, jnp.uint32
HEAD_DIM, WINDOW, DILATION, EPS = 32, 8, 2, 1e-5
LANES, PAD, GROUP = 128, 16, 16

LHS = ((0, 1, 3), (2, 1, 3), (0, 0, 0), (3, 0, 3), (0, 1, 1), (2, -1, 0), (1, -1, 3))
RHS = ((0, 1, 3), (0, 0, 0), (1, -1, 3), (2, -1, 0), (3, 0, 3), (0, 1, 1), (2, 1, 3))
ORDER = (1, 4, 0, 3, 2, 6, 5)
COMPLETES = {3: 2, 2: 1, 6: 0, 5: 3}


def _dot(a, b):
    return jnp.dot(a, b, preferred_element_type=F32)


def _comb(spec, get):
    i, sign, j = spec
    return get(i) if sign == 0 else get(i) + get(j) if sign > 0 else get(i) - get(j)


def _block(s, q):
    return s // 2 + q // 2 * 2, s % 2 + q % 2 * 2


class _Quadrants:
    def __init__(self, slots=None):
        self.slots = {} if slots is None else slots

    def add(self, o, m):
        t, done = self.slots, None
        if o == 1:
            t[0] = m
        elif o == 4:
            t[1] = m
        elif o == 0:
            t[4] = m
        elif o == 3:
            done = t[0] + m
            t[2] = m - t[1]
        elif o == 2:
            done = m + t[1]
            t[3] = m - t[0]
        else:
            done = t[2 if o == 6 else 3] + t[4] + m
        return done


def _two_levels(product, emit, slots):
    inner = _Quadrants(slots(0))
    outer = [_Quadrants(slots(s + 1)) for s in range(4)]
    for o in ORDER:
        for i in ORDER:
            v = inner.add(i, product(o, i))
            if v is not None:
                v = outer[COMPLETES[i]].add(o, v)
                if v is not None:
                    emit(COMPLETES[i], COMPLETES[o], v)


class _Parked:
    def __init__(self, refs, zero):
        self.refs, self.zero = refs, zero

    def __setitem__(self, k, v):
        self.shape = v.shape
        self.refs[k][:v.shape[0], :v.shape[1]] = v

    def __getitem__(self, k):
        return self.refs[k][pl.ds(pl.multiple_of(self.zero * 32, 32), self.shape[0]), :self.shape[1]]


def _identity(v):
    return v


class _SideWork:
    def __init__(self, jobs, first, last, never):
        self.jobs, self.slots, self.done, self.n, self.never = jobs, last - first + 1, 0, -first, never

    def step(self, product):
        self.n += 1
        end = min(len(self.jobs), -(-len(self.jobs) * self.n // self.slots))
        todo = self.jobs[self.done:max(end, self.done)]
        self.done += len(todo)
        rows = product.shape[0] // 8
        for k, job in enumerate(todo):
            col, row = divmod(k * rows * (product.shape[1] // LANES) // len(todo), rows)
            tile = product[8 * row:8 * row + 8, col * LANES:(col + 1) * LANES]

            def after(v, tile=tile):
                t = tile if v.dtype == F32 else pltpu.bitcast(tile, v.dtype)
                return jnp.where(self.never, jnp.concatenate([t] * (v.shape[0] // 8), axis=0), v)

            job(after)


def _rows(start, n):
    if isinstance(start, int):
        return pl.ds(start, n)
    index, step, offset = start
    return pl.ds(pl.multiple_of(index * step, step) + offset, n)


def _half(start):
    return start // 2 if isinstance(start, int) else (start[0], start[1] // 2, start[2] // 2)


def _put(ref, k, r0, cols, v):
    if ref.dtype == BF16:
        ref[k, _rows(r0, v.shape[0]), cols] = v.astype(BF16)
    else:
        ref[k, _rows(_half(r0), v.shape[0] // 2), cols] = pltpu.bitcast(v.astype(BF16), U32)


def _get(ref, k, r0, n, cols=slice(None)):
    if ref.dtype == BF16:
        return ref[k, _rows(r0, n), cols]
    return pltpu.bitcast(ref[k, _rows(_half(r0), n // 2), cols], BF16)


def _operand_buffer(n, rows, cols, words):
    return pltpu.VMEM((n, rows // 2, cols), U32) if words else pltpu.VMEM((n, rows, cols), BF16)


def _split_jobs(spec, load, store):
    blocks = []

    def job(o, after):
        quad = [after(_comb(spec[o], lambda q: blocks[_block(s, q)[0]][_block(s, q)[1]])) for s in range(4)]
        for i in range(7):
            store(7 * o + i, _comb(spec[i], quad.__getitem__))

    return [lambda after: blocks.extend(load(after))] + [functools.partial(job, o) for o in range(7)]


def _swap_block_lane(blocks):
    lane = jax.lax.broadcasted_iota(jnp.int32, blocks[0].shape, 1)
    t = [x if b == 0 else pltpu.roll(x, b, 1) for b, x in enumerate(blocks)]
    s = [t[(-c) % 8] for c in range(8)]
    for bit in (1, 2, 4):
        m = (lane & bit) != 0
        s = [jnp.where(m, s[(c - bit) % 8], s[c]) for c in range(8)]
    return [x if c == 0 else pltpu.roll(x, LANES - c, 1) for c, x in enumerate(s)]


def _attention(qkv, row, n, out):
    rows = [_rows(row[:2] + (row[2] + PAD - DILATION * w,), n) for w in range(WINDOW)]
    logits, p = [], []

    def scores(after):
        pos = jax.lax.broadcasted_iota(jnp.int32, (n, LANES), 0) + (row[0] * row[1] + row[2])
        q = [after(qkv[0, c, rows[0], :]) for c in range(8)]
        for w in range(WINDOW):
            s = functools.reduce(jnp.add, (q[c] * qkv[1, c, rows[w], :] for c in range(8)))
            s = s + pltpu.roll(s, LANES - 8, 1)
            s = s + pltpu.roll(s, LANES - 16, 1)
            s = s * (HEAD_DIM ** -0.5)
            logits.append(jnp.where(pos >= DILATION * w, s, -1e9) if row[2] < DILATION * w else s)

    def softmax(after):
        lane = jax.lax.broadcasted_iota(jnp.int32, (n, LANES), 1)
        m = after(functools.reduce(jnp.maximum, logits))
        e = [jnp.exp(s - m) for s in logits]
        inv = 1.0 / functools.reduce(jnp.add, e)
        for w in range(WINDOW):
            a = e[w] * inv
            a = jnp.where((lane & 24) == 0, a, pltpu.roll(a, 8, 1))
            p.append(jnp.where((lane & 16) == 0, a, pltpu.roll(a, 16, 1)))

    def values(after):
        p[0] = after(p[0])
        out.extend(_swap_block_lane([
            functools.reduce(jnp.add, (p[w] * qkv[2, c, rows[w], :] for w in range(WINDOW))) for c in range(8)]))

    return scores, softmax, values


def _kernel(x_hbm, wqkv_hbm, wo_hbm, wg_hbm, wu_hbm, wd_hbm, out_hbm,
            x_v, wg_v, wu_v, wd_v, a2, wo2, acc, qkv, w_v, a1, o2, tmp, hid, x_sem, w_sem, f_sem, o_sem, *, cfg):
    _, qm, d = x_hbm.shape
    tf = wg_v.shape[2]
    hd, qd, qf = d // 2, d // 4, tf // 4
    nf = wg_hbm.shape[1] // tf

    def f_copies(j, slot):
        c = pl.ds(pl.multiple_of(j * tf, tf), tf)
        return (pltpu.make_async_copy(wg_hbm.at[:, c], wg_v.at[slot], f_sem.at[0, slot]),
                pltpu.make_async_copy(wu_hbm.at[:, c], wu_v.at[slot], f_sem.at[1, slot]),
                pltpu.make_async_copy(wd_hbm.at[c, :], wd_v.at[slot], f_sem.at[2, slot]))

    def projections():
        nb = cfg["nb"]
        br = qm // nb
        steps, pn = cfg["steps"], cfg["pn"]
        xr, wr = br // steps, hd // steps

        def first_copies(g):
            r, k = (_rows(g * n if isinstance(g, int) else (g, n, 0), n) for n in (xr, wr))
            return (pltpu.make_async_copy(wqkv_hbm.at[:, k, pl.ds(0, d)], w_v.at[0, :, k], x_sem.at[1, g]),
                    pltpu.make_async_copy(x_hbm.at[:, r, :], x_v.at[:, r, :], x_sem.at[0, g]))

        def x_copy(g):
            r = _rows(g * br if isinstance(g, int) else (g, br, 0), br)
            return pltpu.make_async_copy(x_hbm.at[:, r, :], x_v.at[:, r, :], w_sem.at[4 + g])

        def w_copy(m):
            cols = pl.ds(pl.multiple_of(m * d, d), d)
            return pltpu.make_async_copy(wqkv_hbm.at[:, :, cols], w_v.at[m % 2], w_sem.at[m])

        wo_copy = pltpu.make_async_copy(wo_hbm, w_v.at[1], w_sem.at[0])

        def permuted_weight(m, i, r0, n, after=_identity):
            return _swap_block_lane([after(pltpu.bitcast(w_v[m, i, _rows(r0, n), c:c + LANES], U32))
                                     for c in range(0, d, LANES)])

        def normalized(q, r0, after=_identity):
            r = _rows(r0, GROUP)
            x = [after(x_v[q, r, c:c + LANES].astype(F32)) for c in range(0, d, LANES)]
            mean = jnp.sum(functools.reduce(jnp.add, x), axis=-1, keepdims=True) * (1.0 / d)
            x = [v - mean for v in x]
            var = jnp.sum(functools.reduce(jnp.add, [v * v for v in x]), axis=-1, keepdims=True) * (1.0 / d)
            rstd = jax.lax.rsqrt(var + EPS)
            hid[q][r, :] = jnp.broadcast_to(mean, (GROUP, LANES))
            hid[4 + q][r, :] = jnp.broadcast_to(rstd, (GROUP, LANES))
            return [v * rstd for v in x]

        def store_projection(m, q, r0, c0, v):
            n = v.shape[0] // 2
            for a in range(2):
                for p in range(0, v.shape[1], LANES):
                    qkv[m, c0 + (q % 2 * v.shape[1] + p) // LANES, _rows((r0[0], r0[1], r0[2] + PAD + (q // 2 * 2 + a) * qm), n), :] = (
                        v[a * n:(a + 1) * n, p:p + LANES])

        def one_level(m, r0, n, c0, rhs, work):
            c = _Quadrants()
            for o in ORDER:
                lhs = jnp.concatenate([_get(a1[o], a, r0, n) for a in range(2)], axis=0)
                p = _dot(lhs, rhs(o))
                for s in work:
                    s.step(p)
                done = c.add(o, p)
                if done is not None:
                    store_projection(m, COMPLETES[o], r0, c0, done)

        for g in range(steps):
            for c in first_copies(g):
                c.start()
        x_copy(1).start()

        def first_body(g, carry):
            for c in first_copies(g):
                c.wait()
            w = [[pltpu.bitcast(v, BF16).astype(F32) for v in permuted_weight(0, i, (g, wr, 0), wr)] for i in range(2)]
            for p in range(4):
                for o in range(7):
                    _put(o2, 2 * o + p // 2, (g, wr, 0), slice(p % 2 * LANES, (p % 2 + 1) * LANES),
                         _comb(RHS[o], lambda q: w[q // 2][q % 2 * 4 + p]))
            for n in range(0, xr, GROUP):
                for a in range(2):
                    xn = [normalized(q, (g, xr, n)) for q in (a, a + 2)]
                    for p in range(4):
                        for o in range(7):
                            _put(a1[o], a, (g, xr, n), slice(p * LANES, (p + 1) * LANES),
                                 _comb(LHS[o], lambda q: xn[q // 2][q % 2 * 4 + p]))
            return carry

        jax.lax.fori_loop(0, steps, first_body, 0)

        def q_body(g, carry):
            pl.when(g < nb - 2)(lambda: x_copy(g + 2).start())
            pl.when(g == nb // 4)(w_copy(1).start)
            pl.when(g == nb // 2)(w_copy(2).start)
            pl.when(g == nb - 1)(wo_copy.start)
            pl.when(g < nb - 1)(lambda: x_copy(g + 1).wait())
            pl.when(g == nb // 2)(w_copy(1).wait)
            pl.when(g == 3 * nb // 4)(w_copy(2).wait)
            nxt, m, part = (g + 1) % nb, g // (nb // 4), g % (nb // 4)

            def permute(i, n, after):
                src = (m == 2).astype(jnp.int32)
                for c, v in enumerate(permuted_weight(src, i, (part, 4 * hd // nb, n), pn, after)):
                    acc[c, m // 3, _rows((part, 2 * hd // nb, (i * hd + n) // 2), pn // 2), :] = pltpu.bitcast(v, F32)

            def normalize(n, a, after):
                for q in (a, a + 2):
                    for p, v in enumerate(normalized(q, (nxt, br, n), after)):
                        tmp[4 * q + p // 2][n:n + GROUP, p % 2 * LANES:(p % 2 + 1) * LANES] = v

            def operand(o, n, a, after):
                r = _rows((g // nb, 32, n), 32)
                for c in range(0, hd, LANES):
                    v = _comb(LHS[o], lambda q: tmp[4 * (a + q // 2 * 2) + q % 2 * 2 + c // qd][r, c % qd:c % qd + LANES])
                    _put(a1[o], a, (nxt, br, n), slice(c, c + LANES), after(v))

            never = g >= nb
            one_level(0, (g, br, 0), br, 0, lambda o: jnp.concatenate([_get(o2, 2 * o + b, 0, hd) for b in range(2)], axis=1), [
                _SideWork([functools.partial(normalize, n, a) for n in range(0, br, GROUP) for a in range(2)],
                          *cfg["norm"], never),
                _SideWork([functools.partial(permute, i, n) for i in range(2) for n in range(0, 4 * hd // nb, pn)],
                          *cfg["perm"], never),
                _SideWork([functools.partial(operand, o, n, a) for o in ORDER for n in range(0, br, 32)
                           for a in range(2)], *cfg["opnd"], never)])
            return carry

        jax.lax.fori_loop(0, nb, q_body, 0)
        nk = cfg["nk"]
        br = qm // nk
        for c in f_copies(0, 0):
            c.start()

        def weight_jobs(load, store, t, n):
            jobs = []
            for m in range(0, n, GROUP):
                for p in range(2):
                    jobs += _split_jobs(
                        RHS,
                        lambda after, m=m, p=p: [[after(load(i, (t, n, m), k, p).astype(F32))
                                                  for k in range(4)] for i in range(4)],
                        lambda k, v, m=m, p=p: store(k, (t, n, m), p, v))
            return jobs

        def wo_jobs(r0, n):
            return weight_jobs(lambda i, r, k, p: w_v[1, i // 2, _rows(r[:2] + (r[2] + i % 2 * qd,), GROUP),
                                                      p * hd + k * LANES:p * hd + (k + 1) * LANES],
                               lambda t, r, p, v: _put(wo2, 2 * t + p, r, slice(None), v), r0, n)

        def k_body(t, carry):
            def load(n, c, after):
                r = _rows((t, br, n), GROUP)
                mean = [after(hid[q][r, :]) for q in range(4)]
                return [[(x_v[q, r, k * qd + c:k * qd + c + LANES].astype(F32) - mean[q]) * hid[4 + q][r, :]
                         for k in range(4)] for q in range(4)]

            jobs = []
            for n in range(0, br, GROUP):
                for c in (0, LANES):
                    jobs += _split_jobs(LHS, functools.partial(load, n, c),
                                        lambda k, v, n=n, c=c: _put(a2, k, (t, br, n), slice(c, c + LANES), v))
            wv_jobs = weight_jobs(lambda i, r, k, p: _get(acc.at[2 * k + p], 1, r[:2] + (r[2] + i * qd,), GROUP),
                                  lambda k, r, p, v: _put(o2, k, r[:2] + (r[2] + p * qd,), slice(0, LANES), v),
                                  t, qd // nk)
            w = [jnp.concatenate([_get(acc.at[q % 2 * 4 + c], 0, q // 2 * hd, hd).astype(F32) for c in range(4)],
                                 axis=1) for q in range(4)]
            one_level(1, (t, br, 0), br, 0, lambda o: _comb(RHS[o], w.__getitem__).astype(BF16),
                      [_SideWork(jobs, *cfg["a2"], t >= 4), _SideWork(wv_jobs, *cfg["wv"], t >= 4)])
            return carry

        jax.lax.fori_loop(0, nk, k_body, 0)
        wo_copy.wait()

        nv = cfg["nv"]
        vr = qm // nv

        def v_body(t, carry):
            def clear(k, after):
                zero = after(jnp.zeros((8, LANES), F32))
                acc[k, t % 2, _rows((t // 2, vr, 0), vr), :] = jnp.tile(zero, (vr // 8, 1))

            never = t >= 2 * nv
            work = [_SideWork([functools.partial(clear, k) for k in range(49)], *cfg["zero"], never),
                    _SideWork(wo_jobs(t, qd // (2 * nv)), *cfg["wo"], never)]

            def product(o, i):
                p = _dot(_get(a2, 7 * o + i, (t // 2, vr, 0), vr), _get(o2, 7 * o + i, (t % 2, qd, 0), qd, slice(0, LANES)))
                for s in work:
                    s.step(p)
                return p

            def emit(s, q, v):
                i, k = _block(s, q)
                qkv[2, 2 * k + t % 2, _rows((t // 2, vr, PAD + i * qm), vr), :] = v

            _two_levels(product, emit, lambda s: None)
            return carry

        jax.lax.fori_loop(0, 2 * nv, v_body, 0, unroll=cfg["vu"])

    projections()

    for m in (1, 2):
        for c in range(8):
            qkv[m, c, :PAD, :] = jnp.broadcast_to(qkv[m, c, PAD:PAD + 1, :], (PAD, LANES))

    def rest():
        groups = -(-qm // (GROUP * nf))

        def ffn_body(j, carry):
            slot = j % 2

            @pl.when(j + 1 < nf)
            def _():
                for c in f_copies(j + 1, 1 - slot):
                    c.start()

            for c in f_copies(j, slot):
                c.wait()

            att, units, jobs = [], [], []
            for n in range(groups if cfg["au"] else 0):
                r0 = (j, (groups - 1) * GROUP, n * GROUP)
                if n == groups - 1:
                    r0 = (jnp.where(j < qm // GROUP - nf * (groups - 1), j, 0), GROUP, nf * (groups - 1) * GROUP)
                an = cfg["an"]
                att.append([[[] for _ in range(0, GROUP, an)] for q in range(4)])
                units += [_attention(qkv, r0[:2] + (r0[2] + q * qm + k,), an, att[n][q][k // an])
                          for q in range(4) for k in range(0, GROUP, an)]
                for p in range(2):
                    jobs += _split_jobs(
                        LHS, lambda after, n=n, p=p: [[jnp.concatenate([v[2 * k + p] for v in att[n][q]], axis=0) for k in range(4)] for q in range(4)],
                        lambda t, v, r0=r0, p=p: _put(o2, t, r0, slice(p * LANES, (p + 1) * LANES), v))
            lag = cfg["lag"]
            stages = [units[u - lag[k]][k] for u in range(len(units) + lag[2]) for k in cfg["so"]
                      if 0 <= u - lag[k] < len(units)]
            if cfg["pace"] is None:
                for job in stages:
                    job(_identity)
                stages = []
            work = _SideWork(jobs, *cfg["att"], j >= nf)
            early = _SideWork(stages, *(cfg["pace"] or (0, 1)), j >= nf)

            def w_in(s, q):
                i, k = _block(s, q)
                r, c = slice(i * qd, (i + 1) * qd), slice(k * qf, (k + 1) * qf)
                return jnp.concatenate([wg_v[slot, r, c].astype(F32), wu_v[slot, r, c].astype(F32)], axis=1)

            def w_out(s, q):
                i, k = _block(s, q)
                return jnp.concatenate([wd_v[slot, i * qf:(i + 1) * qf, c + k * LANES:c + (k + 1) * LANES].astype(F32)
                                        for c in (0, hd)], axis=1)

            def operand(spec, o, i, get):
                return _comb(spec[i], lambda s: _comb(spec[o], lambda q: get(s, q))).astype(BF16)

            h = _Parked(hid, j // nf)

            def gate(s, q, v):
                h[4 * s + q] = v[:, :qf] * v[:, qf:]

            def product(o, i):
                p = _dot(_get(a2, 7 * o + i, 0, qm), operand(RHS, o, i, w_in))
                early.step(p)
                work.step(p)
                return p

            _two_levels(product, gate, lambda s: _Parked(tmp[5 * s:], j // nf) if s in cfg["fpark"] else None)
            for o in cfg["down"][0]:
                for i in cfg["down"][1]:
                    p = _dot(operand(LHS, o, i, lambda s, q: h[4 * s + q]), operand(RHS, o, i, w_out))
                    for c in range(2):
                        acc[7 * o + i, c] += p[:, c * LANES:(c + 1) * LANES]
                    early.step(p)
                    work.step(p)
            return carry

        if not cfg["skip"]:
            jax.lax.fori_loop(0, nf, ffn_body, 0)

        no = cfg["no"]
        rows = qm // no

        def o_copy(t):
            at = (slice(None), _rows(t // 2 * rows if isinstance(t, int) else (t // 2, rows, 0), rows), pl.ds(pl.multiple_of(t % 2 * hd, hd), hd))
            return pltpu.make_async_copy(x_v.at[at], out_hbm.at[at], o_sem.at[t])

        def out_body(t, carry):
            r = _rows(t // 2 * rows if isinstance(t, int) else (t // 2, rows, 0), rows)

            def product(o, i):
                p = _dot(_get(o2, 7 * o + i, (t // 2, rows, 0), rows), _get(wo2, 2 * (7 * o + i) + t % 2, 0, qd))
                return p + acc[7 * o + i, t % 2, r, :]

            def emit(s, q, v):
                i, k = _block(s, q)
                at = (i, r, pl.ds(pl.multiple_of(t % 2 * hd, hd) + k * LANES, LANES))
                x_v[at] = (x_v[at].astype(F32) + v).astype(BF16)

            _two_levels(product, emit,
                        lambda s: _Parked(tmp[5 * s:], t // (2 * no)) if s in cfg["opark"] else None)
            o_copy(t).start()
            return carry

        jax.lax.fori_loop(0, 2 * no, out_body, 0)
        for t in range(2 * no):
            o_copy(t).wait()

    rest()


CONFIG = dict(steps=4, norm=(0, 2), perm=(0, 5), opnd=(5, 6), a2=(0, 5), wv=(5, 6), nv=4, zero=(20, 44), wo=(0, 30),
              words="loa", down=((2, 4, 5, 3, 1, 6, 0), (3, 2, 4, 5, 1, 6, 0)), skip=False, no=4, opark=(), att=(18, 96), vu=1, nk=2, nb=8, an=16, lag=(0, 2, 2), so=(0, 1, 2), pace=None, au=1, fpark=(0, 1, 2, 3, 4), pn=32)


def make(flags={"XLA_TPU_EVENLY_DISTRIBUTE_CRITICAL_NODES": True}, **overrides):
    cfg = dict(CONFIG, **overrides)

    def fn(A_x, A_wqkv, A_wo, B_x, B_w_gate, B_w_up, B_w_down):
        del B_x
        b, s, d = A_x.shape
        qm, tf = s // 4, 4 * LANES
        any_spec = pl.BlockSpec(memory_space=pl.ANY)
        out = pl.pallas_call(
            functools.partial(_kernel, cfg=cfg),
            in_specs=[any_spec] * 6,
            out_specs=any_spec,
            out_shape=jax.ShapeDtypeStruct((4, qm, d), A_x.dtype),
            scratch_shapes=[
                pltpu.VMEM((4, qm, d), BF16),
                pltpu.VMEM((2, d, tf), BF16),
                pltpu.VMEM((2, d, tf), BF16),
                pltpu.VMEM((2, tf, d), BF16),
                _operand_buffer(49, qm, d // 4, True),
                _operand_buffer(98, d // 4, LANES, "o" in cfg["words"]),
                pltpu.VMEM((49, 2, qm, LANES), F32),
                pltpu.VMEM((3, 8, PAD + s, LANES), F32),
                pltpu.VMEM((2, 2, d // 2, d), BF16),
                [_operand_buffer(2, qm, d // 2, "a" in cfg["words"])] * 7,
                _operand_buffer(49, qm, d // 4, "l" in cfg["words"]),
                [pltpu.VMEM((qm, tf // 2), F32)] * 25,
                [pltpu.VMEM((qm, tf // 4), F32)] * 16,
                pltpu.SemaphoreType.DMA((2, cfg["steps"])),
                pltpu.SemaphoreType.DMA((4 + cfg["nb"],)),
                pltpu.SemaphoreType.DMA((3, 2)),
                pltpu.SemaphoreType.DMA((2 * cfg["no"],)),
            ],
            compiler_params=pltpu.CompilerParams(vmem_limit_bytes=126 * 2 ** 20, flags=flags,
                                                 disable_bounds_checks=True),
        )(A_x.reshape(4, qm, d), A_wqkv.reshape(2, d // 2, 3 * d), A_wo.reshape(2, d // 2, d), B_w_gate, B_w_up, B_w_down)
        return out.reshape(b, s, d)
    return fn


@jax.jit
def pallas_parallel_sum__sliding_local_dilated__glu_gated_bilinear__prompt_kernel(
    A_x: jax.Array,
    A_wqkv: jax.Array,
    A_wo: jax.Array,
    B_x: jax.Array,
    B_w_gate: jax.Array,
    B_w_up: jax.Array,
    B_w_down: jax.Array,
):
    return make()(A_x, A_wqkv, A_wo, B_x, B_w_gate, B_w_up, B_w_down)
```

```python
import functools

import jax
import jax.numpy as jnp
import jax.experimental.pallas as pl
import jax.experimental.pallas.tpu as pltpu

F32, BF16, U32 = jnp.float32, jnp.bfloat16, jnp.uint32
HEAD_DIM, WINDOW, DILATION, EPS = 32, 8, 2, 1e-5
LANES, PAD, GROUP = 128, 16, 16

LHS = ((0, 1, 3), (2, 1, 3), (0, 0, 0), (3, 0, 3), (0, 1, 1), (2, -1, 0), (1, -1, 3))
RHS = ((0, 1, 3), (0, 0, 0), (1, -1, 3), (2, -1, 0), (3, 0, 3), (0, 1, 1), (2, 1, 3))
ORDER = (1, 4, 0, 3, 2, 6, 5)
COMPLETES = {3: 2, 2: 1, 6: 0, 5: 3}


def _dot(a, b):
    return jnp.dot(a, b, preferred_element_type=F32)


def _comb(spec, get):
    i, sign, j = spec
    return get(i) if sign == 0 else get(i) + get(j) if sign > 0 else get(i) - get(j)


def _block(s, q):
    return s // 2 + q // 2 * 2, s % 2 + q % 2 * 2


class _Quadrants:
    def __init__(self, slots=None):
        self.slots = {} if slots is None else slots

    def add(self, o, m):
        t, done = self.slots, None
        if o == 1:
            t[0] = m
        elif o == 4:
            t[1] = m
        elif o == 0:
            t[4] = m
        elif o == 3:
            done = t[0] + m
            t[2] = m - t[1]
        elif o == 2:
            done = m + t[1]
            t[3] = m - t[0]
        else:
            done = t[2 if o == 6 else 3] + t[4] + m
        return done


def _two_levels(product, emit, slots):
    inner = _Quadrants(slots(0))
    outer = [_Quadrants(slots(s + 1)) for s in range(4)]
    for o in ORDER:
        for i in ORDER:
            v = inner.add(i, product(o, i))
            if v is not None:
                v = outer[COMPLETES[i]].add(o, v)
                if v is not None:
                    emit(COMPLETES[i], COMPLETES[o], v)


class _Parked:
    def __init__(self, refs, zero):
        self.refs, self.zero = refs, zero

    def __setitem__(self, k, v):
        self.shape = v.shape
        self.refs[k][:v.shape[0], :v.shape[1]] = v

    def __getitem__(self, k):
        return self.refs[k][pl.ds(pl.multiple_of(self.zero * 32, 32), self.shape[0]), :self.shape[1]]


def _identity(v):
    return v


class _SideWork:
    def __init__(self, jobs, first, last, never):
        self.jobs, self.slots, self.done, self.n, self.never = jobs, last - first + 1, 0, -first, never

    def step(self, product):
        self.n += 1
        end = min(len(self.jobs), -(-len(self.jobs) * self.n // self.slots))
        todo = self.jobs[self.done:max(end, self.done)]
        self.done += len(todo)
        rows = product.shape[0] // 8
        for k, job in enumerate(todo):
            col, row = divmod(k * rows * (product.shape[1] // LANES) // len(todo), rows)
            tile = product[8 * row:8 * row + 8, col * LANES:(col + 1) * LANES]

            def after(v, tile=tile):
                t = tile if v.dtype == F32 else pltpu.bitcast(tile, v.dtype)
                return jnp.where(self.never, jnp.concatenate([t] * (v.shape[0] // 8), axis=0), v)

            job(after)


def _rows(start, n):
    if isinstance(start, int):
        return pl.ds(start, n)
    index, step, offset = start
    return pl.ds(pl.multiple_of(index * step, step) + offset, n)


def _half(start):
    return start // 2 if isinstance(start, int) else (start[0], start[1] // 2, start[2] // 2)


def _put(ref, k, r0, cols, v):
    if ref.dtype == BF16:
        ref[k, _rows(r0, v.shape[0]), cols] = v.astype(BF16)
    else:
        ref[k, _rows(_half(r0), v.shape[0] // 2), cols] = pltpu.bitcast(v.astype(BF16), U32)


def _get(ref, k, r0, n, cols=slice(None)):
    if ref.dtype == BF16:
        return ref[k, _rows(r0, n), cols]
    return pltpu.bitcast(ref[k, _rows(_half(r0), n // 2), cols], BF16)


def _operand_buffer(n, rows, cols, words):
    return pltpu.VMEM((n, rows // 2, cols), U32) if words else pltpu.VMEM((n, rows, cols), BF16)


def _split_jobs(spec, load, store):
    blocks = []

    def job(o, after):
        quad = [after(_comb(spec[o], lambda q: blocks[_block(s, q)[0]][_block(s, q)[1]])) for s in range(4)]
        for i in range(7):
            store(7 * o + i, _comb(spec[i], quad.__getitem__))

    return [lambda after: blocks.extend(load(after))] + [functools.partial(job, o) for o in range(7)]


def _swap_block_lane(blocks):
    lane = jax.lax.broadcasted_iota(jnp.int32, blocks[0].shape, 1)
    t = [x if b == 0 else pltpu.roll(x, b, 1) for b, x in enumerate(blocks)]
    s = [t[(-c) % 8] for c in range(8)]
    for bit in (1, 2, 4):
        m = (lane & bit) != 0
        s = [jnp.where(m, s[(c - bit) % 8], s[c]) for c in range(8)]
    return [x if c == 0 else pltpu.roll(x, LANES - c, 1) for c, x in enumerate(s)]


def _attention(qkv, row, n, out):
    rows = [_rows(row[:2] + (row[2] - DILATION * w,), n) for w in range(WINDOW)]
    logits, p = [], []

    def scores(after):
        pos = jax.lax.broadcasted_iota(jnp.int32, (n, LANES), 0) + (row[0] * row[1] + row[2] - PAD)
        q = [after(qkv[0, c, rows[0], :]) for c in range(8)]
        for w in range(WINDOW):
            s = functools.reduce(jnp.add, (q[c] * qkv[1, c, rows[w], :] for c in range(8)))
            s = s + pltpu.roll(s, LANES - 8, 1)
            s = s + pltpu.roll(s, LANES - 16, 1)
            s = s * (HEAD_DIM ** -0.5)
            logits.append(jnp.where(pos >= DILATION * w, s, -1e9) if row[2] - PAD < DILATION * w else s)

    def softmax(after):
        lane = jax.lax.broadcasted_iota(jnp.int32, (n, LANES), 1)
        m = after(functools.reduce(jnp.maximum, logits))
        e = [jnp.exp(s - m) for s in logits]
        inv = 1.0 / functools.reduce(jnp.add, e)
        for w in range(WINDOW):
            a = e[w] * inv
            a = jnp.where((lane & 24) == 0, a, pltpu.roll(a, 8, 1))
            p.append(jnp.where((lane & 16) == 0, a, pltpu.roll(a, 16, 1)))

    def values(after):
        p[0] = after(p[0])
        out.extend(_swap_block_lane([
            functools.reduce(jnp.add, (p[w] * qkv[2, c, rows[w], :] for w in range(WINDOW))) for c in range(8)]))

    return scores, softmax, values


def _kernel(x_hbm, wqkv_hbm, wo_hbm, wg_hbm, wu_hbm, wd_hbm, out_hbm,
            x_v, wg_v, wu_v, wd_v, a2, wo2, acc, qkv, w_v, a1, o2, tmp, hid, x_sem, w_sem, f_sem, o_sem, *, cfg):
    _, qm, d = x_hbm.shape
    tf = wg_v.shape[2]
    hd, qd, qf = d // 2, d // 4, tf // 4
    nf = wg_hbm.shape[1] // tf

    def first_row(q):
        return q * qm + (1 + q // 2) * PAD

    def f_copies(j, slot):
        c = pl.ds(pl.multiple_of(j * tf, tf), tf)
        return (pltpu.make_async_copy(wg_hbm.at[:, c], wg_v.at[slot], f_sem.at[0, slot]),
                pltpu.make_async_copy(wu_hbm.at[:, c], wu_v.at[slot], f_sem.at[1, slot]),
                pltpu.make_async_copy(wd_hbm.at[c, :], wd_v.at[slot], f_sem.at[2, slot]))

    def projections():
        nb = cfg["nb"]
        br = qm // nb
        steps, pn = cfg["steps"], cfg["pn"]
        xr, wr = br // steps, hd // steps

        def first_copies(g):
            r, k = (_rows(g * n if isinstance(g, int) else (g, n, 0), n) for n in (xr, wr))
            return (pltpu.make_async_copy(wqkv_hbm.at[:, k, pl.ds(0, d)], w_v.at[0, :, k], x_sem.at[1, g]),
                    pltpu.make_async_copy(x_hbm.at[:, r, :], x_v.at[:, r, :], x_sem.at[0, g]))

        def x_copy(g):
            r = _rows(g * br if isinstance(g, int) else (g, br, 0), br)
            return pltpu.make_async_copy(x_hbm.at[:, r, :], x_v.at[:, r, :], w_sem.at[4 + g])

        def w_copy(m):
            cols = pl.ds(pl.multiple_of(m * d, d), d)
            return pltpu.make_async_copy(wqkv_hbm.at[:, :, cols], w_v.at[m % 2], w_sem.at[m])

        wo_copy = pltpu.make_async_copy(wo_hbm, w_v.at[1], w_sem.at[0])

        def permuted_weight(m, i, r0, n, after=_identity):
            return _swap_block_lane([after(pltpu.bitcast(w_v[m, i, _rows(r0, n), c:c + LANES], U32))
                                     for c in range(0, d, LANES)])

        def normalized(q, r0, after=_identity):
            r = _rows(r0, GROUP)
            x = [after(x_v[q, r, c:c + LANES].astype(F32)) for c in range(0, d, LANES)]
            mean = jnp.sum(functools.reduce(jnp.add, x), axis=-1, keepdims=True) * (1.0 / d)
            x = [v - mean for v in x]
            var = jnp.sum(functools.reduce(jnp.add, [v * v for v in x]), axis=-1, keepdims=True) * (1.0 / d)
            rstd = jax.lax.rsqrt(var + EPS)
            hid[q][r, :] = jnp.broadcast_to(mean, (GROUP, LANES))
            hid[4 + q][r, :] = jnp.broadcast_to(rstd, (GROUP, LANES))
            return [v * rstd for v in x]

        def store_projection(m, q, r0, c0, v):
            n = v.shape[0] // 2
            for a in range(2):
                for p in range(0, v.shape[1], LANES):
                    qkv[m, c0 + (q % 2 * v.shape[1] + p) // LANES, _rows((r0[0], r0[1], r0[2] + first_row(q // 2 * 2 + a)), n), :] = (
                        v[a * n:(a + 1) * n, p:p + LANES])

        def one_level(m, r0, n, c0, rhs, work):
            c = _Quadrants()
            for o in ORDER:
                lhs = jnp.concatenate([_get(a1[o], a, r0, n) for a in range(2)], axis=0)
                p = _dot(lhs, rhs(o))
                for s in work:
                    s.step(p)
                done = c.add(o, p)
                if done is not None:
                    store_projection(m, COMPLETES[o], r0, c0, done)

        for g in range(steps):
            for c in first_copies(g):
                c.start()
        x_copy(1).start()

        def first_body(g, carry):
            for c in first_copies(g):
                c.wait()
            w = [[pltpu.bitcast(v, BF16).astype(F32) for v in permuted_weight(0, i, (g, wr, 0), wr)] for i in range(2)]
            for p in range(4):
                for o in range(7):
                    _put(o2, 2 * o + p // 2, (g, wr, 0), slice(p % 2 * LANES, (p % 2 + 1) * LANES),
                         _comb(RHS[o], lambda q: w[q // 2][q % 2 * 4 + p]))
            for n in range(0, xr, GROUP):
                for a in range(2):
                    xn = [normalized(q, (g, xr, n)) for q in (a, a + 2)]
                    for p in range(4):
                        for o in range(7):
                            _put(a1[o], a, (g, xr, n), slice(p * LANES, (p + 1) * LANES),
                                 _comb(LHS[o], lambda q: xn[q // 2][q % 2 * 4 + p]))
            return carry

        jax.lax.fori_loop(0, steps, first_body, 0)

        def q_body(g, carry):
            pl.when(g < nb - 2)(lambda: x_copy(g + 2).start())
            pl.when(g == nb // 4)(w_copy(1).start)
            pl.when(g == nb // 2)(w_copy(2).start)
            pl.when(g == nb - 1)(wo_copy.start)
            pl.when(g < nb - 1)(lambda: x_copy(g + 1).wait())
            pl.when(g == nb // 2)(w_copy(1).wait)
            pl.when(g == 3 * nb // 4)(w_copy(2).wait)
            nxt, m, part = (g + 1) % nb, g // (nb // 4), g % (nb // 4)

            def permute(i, n, after):
                src = (m == 2).astype(jnp.int32)
                for c, v in enumerate(permuted_weight(src, i, (part, 4 * hd // nb, n), pn, after)):
                    acc[c, m // 3, _rows((part, 2 * hd // nb, (i * hd + n) // 2), pn // 2), :] = pltpu.bitcast(v, F32)

            def normalize(n, a, after):
                for q in (a, a + 2):
                    for p, v in enumerate(normalized(q, (nxt, br, n), after)):
                        tmp[4 * q + p // 2][n:n + GROUP, p % 2 * LANES:(p % 2 + 1) * LANES] = v

            def operand(o, n, a, after):
                r = _rows((g // nb, 32, n), 32)
                for c in range(0, hd, LANES):
                    v = _comb(LHS[o], lambda q: tmp[4 * (a + q // 2 * 2) + q % 2 * 2 + c // qd][r, c % qd:c % qd + LANES])
                    _put(a1[o], a, (nxt, br, n), slice(c, c + LANES), after(v))

            never = g >= nb
            one_level(0, (g, br, 0), br, 0, lambda o: jnp.concatenate([_get(o2, 2 * o + b, 0, hd) for b in range(2)], axis=1), [
                _SideWork([functools.partial(normalize, n, a) for n in range(0, br, GROUP) for a in range(2)],
                          *cfg["norm"], never),
                _SideWork([functools.partial(permute, i, n) for i in range(2) for n in range(0, 4 * hd // nb, pn)],
                          *cfg["perm"], never),
                _SideWork([functools.partial(operand, o, n, a) for o in ORDER for n in range(0, br, 32)
                           for a in range(2)], *cfg["opnd"], never)])
            return carry

        jax.lax.fori_loop(0, nb, q_body, 0)
        nk = cfg["nk"]
        br = qm // nk
        for c in f_copies(0, 0):
            c.start()

        def weight_jobs(load, store, t, n):
            jobs = []
            for m in range(0, n, GROUP):
                for p in range(2):
                    jobs += _split_jobs(
                        RHS,
                        lambda after, m=m, p=p: [[after(load(i, (t, n, m), k, p).astype(F32))
                                                  for k in range(4)] for i in range(4)],
                        lambda k, v, m=m, p=p: store(k, (t, n, m), p, v))
            return jobs

        def wo_jobs(r0, n):
            return weight_jobs(lambda i, r, k, p: w_v[1, i // 2, _rows(r[:2] + (r[2] + i % 2 * qd,), GROUP),
                                                      p * hd + k * LANES:p * hd + (k + 1) * LANES],
                               lambda t, r, p, v: _put(wo2, 2 * t + p, r, slice(None), v), r0, n)

        def k_body(t, carry):
            def load(n, c, after):
                r = _rows((t, br, n), GROUP)
                mean = [after(hid[q][r, :]) for q in range(4)]
                return [[(x_v[q, r, k * qd + c:k * qd + c + LANES].astype(F32) - mean[q]) * hid[4 + q][r, :]
                         for k in range(4)] for q in range(4)]

            jobs = []
            for n in range(0, br, GROUP):
                for c in (0, LANES):
                    jobs += _split_jobs(LHS, functools.partial(load, n, c),
                                        lambda k, v, n=n, c=c: _put(a2, k, (t, br, n), slice(c, c + LANES), v))
            wv_jobs = weight_jobs(lambda i, r, k, p: _get(acc.at[2 * k + p], 1, r[:2] + (r[2] + i * qd,), GROUP),
                                  lambda k, r, p, v: _put(o2, k, r[:2] + (r[2] + p * qd,), slice(0, LANES), v),
                                  t, qd // nk)
            w = [jnp.concatenate([_get(acc.at[q % 2 * 4 + c], 0, q // 2 * hd, hd).astype(F32) for c in range(4)],
                                 axis=1) for q in range(4)]
            one_level(1, (t, br, 0), br, 0, lambda o: _comb(RHS[o], w.__getitem__).astype(BF16),
                      [_SideWork(jobs, *cfg["a2"], t >= 4), _SideWork(wv_jobs, *cfg["wv"], t >= 4)])
            return carry

        jax.lax.fori_loop(0, nk, k_body, 0)
        wo_copy.wait()

        nv = cfg["nv"]
        vr = qm // nv

        def v_body(t, carry):
            def clear(k, after):
                zero = after(jnp.zeros((8, LANES), F32))
                acc[k, t % 2, _rows((t // 2, vr, 0), vr), :] = jnp.tile(zero, (vr // 8, 1))

            never = t >= 2 * nv
            work = [_SideWork([functools.partial(clear, k) for k in range(49)], *cfg["zero"], never),
                    _SideWork(wo_jobs(t, qd // (2 * nv)), *cfg["wo"], never)]

            def product(o, i):
                p = _dot(_get(a2, 7 * o + i, (t // 2, vr, 0), vr), _get(o2, 7 * o + i, (t % 2, qd, 0), qd, slice(0, LANES)))
                for s in work:
                    s.step(p)
                return p

            def emit(s, q, v):
                i, k = _block(s, q)
                qkv[2, 2 * k + t % 2, _rows((t // 2, vr, first_row(i)), vr), :] = v

            _two_levels(product, emit, lambda s: None)
            return carry

        jax.lax.fori_loop(0, 2 * nv, v_body, 0, unroll=cfg["vu"])

    projections()

    for m in (1, 2):
        for c in range(8):
            qkv[m, c, :PAD, :] = jnp.broadcast_to(qkv[m, c, PAD:PAD + 1, :], (PAD, LANES))
            qkv[m, c, first_row(2) - PAD:first_row(2), :] = qkv[m, c, first_row(2) - 2 * PAD:first_row(2) - PAD, :]

    def rest():
        groups = -(-qm // (GROUP * nf))

        def ffn_body(j, carry):
            slot = j % 2

            @pl.when(j + 1 < nf)
            def _():
                for c in f_copies(j + 1, 1 - slot):
                    c.start()

            for c in f_copies(j, slot):
                c.wait()

            att, units, jobs = [], [], []
            for n in range(groups if cfg["au"] else 0):
                r0 = (j, (groups - 1) * GROUP, n * GROUP)
                rows, swap = [r0[:2] + (r0[2] + first_row(q),) for q in range(4)], None
                if n == groups - 1:
                    g = jnp.where(j < qm // GROUP - nf * (groups - 1), j, 0)
                    r0, swap = (g, GROUP, nf * (groups - 1) * GROUP), g % 2
                    shift = swap * (first_row(2) - first_row(0)) // GROUP
                    rows = [((g + shift if q < 2 else g - shift) // 2, 2 * GROUP, r0[2] + first_row(q))
                            for q in range(4)]
                att.append([[] for q in range(4)])
                units += [_attention(qkv, rows[q], GROUP, att[n][q]) for q in range(4)]

                def load(after, n, p, swap):
                    return [[att[n][q][2 * k + p] if swap is None else
                             jnp.where(swap == 1, att[n][q ^ 2][2 * k + p], att[n][q][2 * k + p])
                             for k in range(4)] for q in range(4)]

                for p in range(2):
                    jobs += _split_jobs(
                        LHS, functools.partial(load, n=n, p=p, swap=swap),
                        lambda t, v, r0=r0, p=p: _put(o2, t, r0, slice(p * LANES, (p + 1) * LANES), v))
            lag = cfg["lag"]
            stages = [units[u - lag[k]][k] for u in range(len(units) + lag[2]) for k in cfg["so"]
                      if 0 <= u - lag[k] < len(units)]
            if cfg["pace"] is None:
                for job in stages:
                    job(_identity)
                stages = []
            work = _SideWork(jobs, *cfg["att"], j >= nf)
            early = _SideWork(stages, *(cfg["pace"] or (0, 1)), j >= nf)

            def w_in(s, q):
                i, k = _block(s, q)
                r, c = slice(i * qd, (i + 1) * qd), slice(k * qf, (k + 1) * qf)
                return jnp.concatenate([wg_v[slot, r, c].astype(F32), wu_v[slot, r, c].astype(F32)], axis=1)

            def w_out(s, q):
                i, k = _block(s, q)
                return jnp.concatenate([wd_v[slot, i * qf:(i + 1) * qf, c + k * LANES:c + (k + 1) * LANES].astype(F32)
                                        for c in (0, hd)], axis=1)

            def operand(spec, o, i, get):
                return _comb(spec[i], lambda s: _comb(spec[o], lambda q: get(s, q))).astype(BF16)

            h = _Parked(hid, j // nf)

            def gate(s, q, v):
                h[4 * s + q] = v[:, :qf] * v[:, qf:]

            def product(o, i):
                p = _dot(_get(a2, 7 * o + i, 0, qm), operand(RHS, o, i, w_in))
                early.step(p)
                work.step(p)
                return p

            _two_levels(product, gate, lambda s: _Parked(tmp[5 * s:], j // nf) if s in cfg["fpark"] else None)
            for o in cfg["down"][0]:
                for i in cfg["down"][1]:
                    p = _dot(operand(LHS, o, i, lambda s, q: h[4 * s + q]), operand(RHS, o, i, w_out))
                    for c in range(2):
                        acc[7 * o + i, c] += p[:, c * LANES:(c + 1) * LANES]
                    early.step(p)
                    work.step(p)
            return carry

        if not cfg["skip"]:
            jax.lax.fori_loop(0, nf, ffn_body, 0)

        no = cfg["no"]
        rows = qm // no

        def o_copy(t):
            at = (slice(None), _rows(t // 2 * rows if isinstance(t, int) else (t // 2, rows, 0), rows), pl.ds(pl.multiple_of(t % 2 * hd, hd), hd))
            return pltpu.make_async_copy(x_v.at[at], out_hbm.at[at], o_sem.at[t])

        def out_body(t, carry):
            r = _rows(t // 2 * rows if isinstance(t, int) else (t // 2, rows, 0), rows)

            def product(o, i):
                p = _dot(_get(o2, 7 * o + i, (t // 2, rows, 0), rows), _get(wo2, 2 * (7 * o + i) + t % 2, 0, qd))
                return p + acc[7 * o + i, t % 2, r, :]

            def emit(s, q, v):
                i, k = _block(s, q)
                at = (i, r, pl.ds(pl.multiple_of(t % 2 * hd, hd) + k * LANES, LANES))
                x_v[at] = (x_v[at].astype(F32) + v).astype(BF16)

            _two_levels(product, emit,
                        lambda s: _Parked(tmp[5 * s:], t // (2 * no)) if s in cfg["opark"] else None)
            o_copy(t).start()
            return carry

        jax.lax.fori_loop(0, 2 * no, out_body, 0)
        for t in range(2 * no):
            o_copy(t).wait()

    rest()


CONFIG = dict(steps=4, norm=(0, 2), perm=(0, 5), opnd=(5, 6), a2=(0, 5), wv=(5, 6), nv=4, zero=(20, 44), wo=(0, 30),
              words="loa", down=((2, 4, 5, 3, 1, 6, 0), (3, 2, 4, 5, 1, 6, 0)), skip=False, no=4, opark=(), att=(18, 96), vu=1, xr=40, nk=2, nb=8, an=16, lag=(0, 2, 2), so=(0, 1, 2), pace=None, au=1, fpark=(0, 1, 2, 3, 4), pn=32)


def make(flags={"XLA_TPU_EVENLY_DISTRIBUTE_CRITICAL_NODES": True}, **overrides):
    cfg = dict(CONFIG, **overrides)

    def fn(A_x, A_wqkv, A_wo, B_x, B_w_gate, B_w_up, B_w_down):
        del B_x
        b, s, d = A_x.shape
        qm, tf = s // 4, 4 * LANES
        any_spec = pl.BlockSpec(memory_space=pl.ANY)
        out = pl.pallas_call(
            functools.partial(_kernel, cfg=cfg),
            in_specs=[any_spec] * 6,
            out_specs=any_spec,
            out_shape=jax.ShapeDtypeStruct((4, qm, d), A_x.dtype),
            scratch_shapes=[
                pltpu.VMEM((4, qm, d), BF16),
                pltpu.VMEM((2, d, tf), BF16),
                pltpu.VMEM((2, d, tf), BF16),
                pltpu.VMEM((2, tf, d), BF16),
                _operand_buffer(49, qm, d // 4, True),
                _operand_buffer(98, d // 4, LANES, "o" in cfg["words"]),
                pltpu.VMEM((49, 2, qm, LANES), F32),
                pltpu.VMEM((3, 8, s + cfg["xr"], LANES), F32),
                pltpu.VMEM((2, 2, d // 2, d), BF16),
                [_operand_buffer(2, qm, d // 2, "a" in cfg["words"])] * 7,
                _operand_buffer(49, qm, d // 4, "l" in cfg["words"]),
                [pltpu.VMEM((qm, tf // 2), F32)] * 25,
                [pltpu.VMEM((qm, tf // 4), F32)] * 16,
                pltpu.SemaphoreType.DMA((2, cfg["steps"])),
                pltpu.SemaphoreType.DMA((4 + cfg["nb"],)),
                pltpu.SemaphoreType.DMA((3, 2)),
                pltpu.SemaphoreType.DMA((2 * cfg["no"],)),
            ],
            compiler_params=pltpu.CompilerParams(vmem_limit_bytes=126 * 2 ** 20, flags=flags,
                                                 disable_bounds_checks=True),
        )(A_x.reshape(4, qm, d), A_wqkv.reshape(2, d // 2, 3 * d), A_wo.reshape(2, d // 2, d), B_w_gate, B_w_up, B_w_down)
        return out.reshape(b, s, d)
    return fn


@jax.jit
def pallas_parallel_sum__sliding_local_dilated__glu_gated_bilinear__prompt_kernel(
    A_x: jax.Array,
    A_wqkv: jax.Array,
    A_wo: jax.Array,
    B_x: jax.Array,
    B_w_gate: jax.Array,
    B_w_up: jax.Array,
    B_w_down: jax.Array,
):
    return make(pn=16, norm=(0,3), perm=(0,5), opnd=(5,6), a2=(0,6), wv=(4,6), zero=(28,46), wo=(2,28))(A_x, A_wqkv, A_wo, B_x, B_w_gate, B_w_up, B_w_down)
```

```python
import functools

import jax
import jax.numpy as jnp
import jax.experimental.pallas as pl
import jax.experimental.pallas.tpu as pltpu

F32, BF16, U32 = jnp.float32, jnp.bfloat16, jnp.uint32
HEAD_DIM, WINDOW, DILATION, EPS = 32, 8, 2, 1e-5
LANES = 128
GROUP = 16
HALO = 16
FIRST_STEPS, Q_STEPS, K_STEPS, V_STEPS, OUT_STEPS = 4, 8, 2, 8, 8

LHS = ((0, 1, 3), (2, 1, 3), (0, 0, 0), (3, 0, 3), (0, 1, 1), (2, -1, 0), (1, -1, 3))
RHS = ((0, 1, 3), (0, 0, 0), (1, -1, 3), (2, -1, 0), (3, 0, 3), (0, 1, 1), (2, 1, 3))
ORDER = (1, 4, 0, 3, 2, 6, 5)
COMPLETES = {3: 2, 2: 1, 6: 0, 5: 3}


def _dot(a, b):
    return jnp.dot(a, b, preferred_element_type=F32)


def _lanes(p):
    return slice(p * LANES, (p + 1) * LANES)


def _identity(v):
    return v


def _comb(spec, get):
    i, sign, j = spec
    return get(i) if sign == 0 else get(i) + get(j) if sign > 0 else get(i) - get(j)


def _block(s, q):
    return s // 2 + q // 2 * 2, s % 2 + q % 2 * 2


class _Quadrants:
    def __init__(self, slots=None):
        self.slots = {} if slots is None else slots

    def add(self, o, m):
        t, done = self.slots, None
        if o == 1:
            t[0] = m
        elif o == 4:
            t[1] = m
        elif o == 0:
            t[4] = m
        elif o == 3:
            done = t[0] + m
            t[2] = m - t[1]
        elif o == 2:
            done = m + t[1]
            t[3] = m - t[0]
        else:
            done = t[2 if o == 6 else 3] + t[4] + m
        return done


def _two_levels(product, emit, slots=lambda k: None):
    inner = _Quadrants(slots(0))
    outer = [_Quadrants(slots(s + 1)) for s in range(4)]
    for o in ORDER:
        for i in ORDER:
            v = inner.add(i, product(o, i))
            if v is not None:
                v = outer[COMPLETES[i]].add(o, v)
                if v is not None:
                    emit(COMPLETES[i], COMPLETES[o], v)


def _split_jobs(spec, load, store):
    blocks = []

    def job(o, after):
        quad = [after(_comb(spec[o], lambda q: blocks[_block(s, q)[0]][_block(s, q)[1]])) for s in range(4)]
        for i in range(7):
            store(7 * o + i, _comb(spec[i], quad.__getitem__))

    return [lambda after: blocks.extend(load(after))] + [functools.partial(job, o) for o in range(7)]


class _Parked:
    def __init__(self, refs, zero):
        self.refs, self.zero = refs, zero

    def __setitem__(self, k, v):
        self.refs[k][...] = v

    def __getitem__(self, k):
        return self.refs[k][_rows((self.zero, 32, 0), self.refs[k].shape[0]), :]


class _SideWork:
    def __init__(self, jobs, first, last, never):
        self.jobs, self.slots, self.done, self.n, self.never = jobs, last - first + 1, 0, -first, never

    def step(self, product):
        self.n += 1
        end = min(len(self.jobs), -(-len(self.jobs) * self.n // self.slots))
        todo = self.jobs[self.done:max(end, self.done)]
        self.done += len(todo)
        rows = product.shape[0] // 8
        for k, job in enumerate(todo):
            col, row = divmod(k * rows * (product.shape[1] // LANES) // len(todo), rows)
            job(functools.partial(self._after, product[8 * row:8 * row + 8, _lanes(col)]))

    def _after(self, tile, v):
        tile = tile if v.dtype == F32 else pltpu.bitcast(tile, v.dtype)
        return jnp.where(self.never, jnp.concatenate([tile] * (v.shape[0] // 8), axis=0), v)


def _rows(start, n):
    if isinstance(start, int):
        return pl.ds(start, n)
    index, step, offset = start
    if isinstance(index, int):
        return pl.ds(index * step + offset, n)
    return pl.ds(pl.multiple_of(index * step, step) + offset, n)


def _plus(start, offset):
    return start[0], start[1], start[2] + offset


def _words(start, n):
    return _rows(start // 2 if isinstance(start, int) else (start[0], start[1] // 2, start[2] // 2), n // 2)


def _put(ref, k, start, cols, v):
    ref[k, _words(start, v.shape[0]), cols] = pltpu.bitcast(v.astype(BF16), U32)


def _get(ref, k, start, n, cols=slice(None)):
    return pltpu.bitcast(ref[k, _words(start, n), cols], BF16)


def _swap_block_lane(blocks):
    lane = jax.lax.broadcasted_iota(jnp.int32, blocks[0].shape, 1)
    t = [x if b == 0 else pltpu.roll(x, b, 1) for b, x in enumerate(blocks)]
    s = [t[(-c) % 8] for c in range(8)]
    for bit in (1, 2, 4):
        m = (lane & bit) != 0
        s = [jnp.where(m, s[(c - bit) % 8], s[c]) for c in range(8)]
    return [x if c == 0 else pltpu.roll(x, LANES - c, 1) for c, x in enumerate(s)]


def _attention(qkv, start, out):
    rows = [_rows(_plus(start, -DILATION * w), GROUP) for w in range(WINDOW)]
    logits, p = [], []

    def scores():
        pos = jax.lax.broadcasted_iota(jnp.int32, (GROUP, LANES), 0) + (start[0] * start[1] + start[2] - HALO)
        q = [qkv[0, c, rows[0], :] for c in range(8)]
        for w in range(WINDOW):
            s = functools.reduce(jnp.add, (q[c] * qkv[1, c, rows[w], :] for c in range(8)))
            s = s + pltpu.roll(s, LANES - 8, 1)
            s = s + pltpu.roll(s, LANES - 16, 1)
            s = s * (HEAD_DIM ** -0.5)
            logits.append(jnp.where(pos >= DILATION * w, s, -1e9) if start[2] - HALO < DILATION * w else s)

    def softmax():
        lane = jax.lax.broadcasted_iota(jnp.int32, (GROUP, LANES), 1)
        m = functools.reduce(jnp.maximum, logits)
        e = [jnp.exp(s - m) for s in logits]
        inv = 1.0 / functools.reduce(jnp.add, e)
        for w in range(WINDOW):
            a = e[w] * inv
            a = jnp.where((lane & 24) == 0, a, pltpu.roll(a, 8, 1))
            p.append(jnp.where((lane & 16) == 0, a, pltpu.roll(a, 16, 1)))

    def values():
        out.extend(_swap_block_lane([
            functools.reduce(jnp.add, (p[w] * qkv[2, c, rows[w], :] for w in range(WINDOW))) for c in range(8)]))

    return scores, softmax, values


def _kernel(x_hbm, wqkv_hbm, wo_hbm, wg_hbm, wu_hbm, wd_hbm, out_hbm,
            x_v, wg_v, wu_v, wd_v, a2, wo2, acc, qkv, w_v, a1, o2, tmp, hid, first_sem, w_sem, f_sem, o_sem):
    _, qm, d = x_hbm.shape
    tf = wg_v.shape[2]
    hd, qd, qf = d // 2, d // 4, tf // 4
    nf = wg_hbm.shape[1] // tf
    q_rows, k_rows, v_rows, out_rows = qm // Q_STEPS, qm // K_STEPS, 2 * qm // V_STEPS, 2 * qm // OUT_STEPS
    x_rows, w_rows = q_rows // FIRST_STEPS, hd // FIRST_STEPS
    mean_v, rstd_v = hid[:4], hid[4:8]

    def first_row(q):
        return q * qm + (1 + q // 2) * HALO

    def first_copies(g):
        r, k = _rows((g, x_rows, 0), x_rows), _rows((g, w_rows, 0), w_rows)
        return (pltpu.make_async_copy(wqkv_hbm.at[:, k, pl.ds(0, d)], w_v.at[0, :, k], first_sem.at[1, g]),
                pltpu.make_async_copy(x_hbm.at[:, r, :], x_v.at[:, r, :], first_sem.at[0, g]))

    def x_copy(g):
        r = _rows((g, q_rows, 0), q_rows)
        return pltpu.make_async_copy(x_hbm.at[:, r, :], x_v.at[:, r, :], w_sem.at[2 + g])

    def f_copies(j, slot):
        c = _rows((j, tf, 0), tf)
        return (pltpu.make_async_copy(wg_hbm.at[:, c], wg_v.at[slot], f_sem.at[0, slot]),
                pltpu.make_async_copy(wu_hbm.at[:, c], wu_v.at[slot], f_sem.at[1, slot]),
                pltpu.make_async_copy(wd_hbm.at[c, :], wd_v.at[slot], f_sem.at[2, slot]))

    def out_copy(t):
        at = (slice(None), _rows((t // 2, out_rows, 0), out_rows), _rows((t % 2, hd, 0), hd))
        return pltpu.make_async_copy(x_v.at[at], out_hbm.at[at], o_sem.at[t])

    wk_copy = pltpu.make_async_copy(wqkv_hbm.at[:, :, pl.ds(d, d)], w_v.at[1], w_sem.at[1])
    wv_copy = pltpu.make_async_copy(wqkv_hbm.at[:, :, pl.ds(2 * d, d)], w_v.at[0], w_sem.at[2])
    wo_copy = pltpu.make_async_copy(wo_hbm, w_v.at[1], w_sem.at[0])

    def permuted_weight(slot, i, start, n, after=_identity):
        return _swap_block_lane([after(pltpu.bitcast(w_v[slot, i, _rows(start, n), _lanes(c)], U32))
                                 for c in range(8)])

    def normalized(q, start, after=_identity):
        r = _rows(start, GROUP)
        x = [after(x_v[q, r, _lanes(c)].astype(F32)) for c in range(8)]
        mean = jnp.sum(functools.reduce(jnp.add, x), axis=-1, keepdims=True) * (1.0 / d)
        x = [v - mean for v in x]
        var = jnp.sum(functools.reduce(jnp.add, [v * v for v in x]), axis=-1, keepdims=True) * (1.0 / d)
        rstd = jax.lax.rsqrt(var + EPS)
        mean_v[q][r, :] = jnp.broadcast_to(mean, (GROUP, LANES))
        rstd_v[q][r, :] = jnp.broadcast_to(rstd, (GROUP, LANES))
        return [v * rstd for v in x]

    def one_level(m, start, n, rhs, work):
        quadrants = _Quadrants()
        for o in ORDER:
            p = _dot(jnp.concatenate([_get(a1[o], a, start, n) for a in range(2)], axis=0), rhs(o))
            for s in work:
                s.step(p)
            v = quadrants.add(o, p)
            if v is not None:
                i, k = divmod(COMPLETES[o], 2)
                for a in range(2):
                    for c in range(4):
                        qkv[m, 4 * k + c, _rows(_plus(start, first_row(2 * i + a)), n), :] = (
                            v[a * n:(a + 1) * n, _lanes(c)])

    def weight_jobs(load, store, t, n):
        jobs = []
        for r in range(0, n, GROUP):
            for p in range(2):
                jobs += _split_jobs(
                    RHS,
                    lambda after, r=r, p=p: [[after(load(i, (t, n, r), k, p).astype(F32)) for k in range(4)]
                                             for i in range(4)],
                    lambda k, v, r=r, p=p: store(k, (t, n, r), p, v))
        return jobs

    for g in range(FIRST_STEPS):
        for c in first_copies(g):
            c.start()
    x_copy(1).start()

    def first_body(g, carry):
        for c in first_copies(g):
            c.wait()
        w = [[pltpu.bitcast(v, BF16).astype(F32) for v in permuted_weight(0, i, (g, w_rows, 0), w_rows)]
             for i in range(2)]
        for c in range(4):
            for o in range(7):
                _put(o2, 2 * o + c // 2, (g, w_rows, 0), _lanes(c % 2),
                     _comb(RHS[o], lambda q: w[q // 2][q % 2 * 4 + c]))
        for a in range(2):
            xn = [normalized(q, (g, x_rows, 0)) for q in (a, a + 2)]
            for c in range(4):
                for o in range(7):
                    _put(a1[o], a, (g, x_rows, 0), _lanes(c), _comb(LHS[o], lambda q: xn[q // 2][q % 2 * 4 + c]))
        return carry

    jax.lax.fori_loop(0, FIRST_STEPS, first_body, 0)

    def q_body(g, carry):
        pl.when(g < Q_STEPS - 2)(lambda: x_copy(g + 2).start())
        pl.when(g == 2)(wk_copy.start)
        pl.when(g == 4)(wv_copy.start)
        pl.when(g == 7)(wo_copy.start)
        pl.when(g < Q_STEPS - 1)(lambda: x_copy(g + 1).wait())
        pl.when(g == 4)(wk_copy.wait)
        pl.when(g == 6)(wv_copy.wait)
        nxt, m, part = (g + 1) % Q_STEPS, g // 2, g % 2

        def permute(i, r, after):
            for c, v in enumerate(permuted_weight((m == 2).astype(jnp.int32), i, (part, qd, r), GROUP, after)):
                acc[c, m // 3, _words((part, qd, i * hd + r), GROUP), :] = pltpu.bitcast(v, F32)

        def normalize(r, a, after):
            for q in (a, a + 2):
                for c, v in enumerate(normalized(q, (nxt, q_rows, r), after)):
                    tmp[4 * q + c // 2][r:r + GROUP, _lanes(c % 2)] = v

        def operand(o, r, a, after):
            rows = _rows((g // Q_STEPS, 32, r), 32)
            for c in range(4):
                v = _comb(LHS[o], lambda q: tmp[4 * (a + q // 2 * 2) + q % 2 * 2 + c // 2][rows, _lanes(c % 2)])
                _put(a1[o], a, (nxt, q_rows, r), _lanes(c), after(v))

        never = g >= Q_STEPS
        one_level(0, (g, q_rows, 0), q_rows,
                  lambda o: jnp.concatenate([_get(o2, 2 * o + b, 0, hd) for b in range(2)], axis=1), [
            _SideWork([functools.partial(normalize, r, a) for r in range(0, q_rows, GROUP) for a in range(2)],
                      0, 3, never),
            _SideWork([functools.partial(permute, i, r) for i in range(2) for r in range(0, qd, GROUP)], 0, 5, never),
            _SideWork([functools.partial(operand, o, r, a) for o in ORDER for r in range(0, q_rows, 32)
                       for a in range(2)], 5, 6, never)])
        return carry

    jax.lax.fori_loop(0, Q_STEPS, q_body, 0)
    for c in f_copies(0, 0):
        c.start()

    def k_body(t, carry):
        def load(r, p, after):
            rows = _rows((t, k_rows, r), GROUP)
            mean = [after(mean_v[q][rows, :]) for q in range(4)]
            return [[(x_v[q, rows, _lanes(2 * k + p)].astype(F32) - mean[q]) * rstd_v[q][rows, :]
                     for k in range(4)] for q in range(4)]

        jobs = []
        for r in range(0, k_rows, GROUP):
            for p in range(2):
                jobs += _split_jobs(LHS, functools.partial(load, r, p),
                                    lambda k, v, r=r, p=p: _put(a2, k, (t, k_rows, r), _lanes(p), v))
        wv_jobs = weight_jobs(lambda i, r, k, p: _get(acc.at[2 * k + p], 1, _plus(r, i * qd), GROUP),
                              lambda k, r, p, v: _put(o2, k, _plus(r, p * qd), _lanes(0), v), t, qd // K_STEPS)
        w = [jnp.concatenate([_get(acc.at[q % 2 * 4 + c], 0, q // 2 * hd, hd).astype(F32) for c in range(4)], axis=1)
             for q in range(4)]
        one_level(1, (t, k_rows, 0), k_rows, lambda o: _comb(RHS[o], w.__getitem__).astype(BF16),
                  [_SideWork(jobs, 0, 6, t >= K_STEPS), _SideWork(wv_jobs, 4, 6, t >= K_STEPS)])
        return carry

    jax.lax.fori_loop(0, K_STEPS, k_body, 0)
    wo_copy.wait()

    def v_body(t, carry):
        start, half = (t // 2, v_rows, 0), t % 2

        def clear(k, after):
            acc[k, half, _rows(start, v_rows), :] = jnp.tile(after(jnp.zeros((8, LANES), F32)), (v_rows // 8, 1))

        wo_jobs = weight_jobs(lambda i, r, k, p: w_v[1, i // 2, _rows(_plus(r, i % 2 * qd), GROUP), _lanes(4 * p + k)],
                              lambda k, r, p, v: _put(wo2, 2 * k + p, r, slice(None), v), t, qd // V_STEPS)
        work = [_SideWork([functools.partial(clear, k) for k in range(49)], 28, 46, t >= V_STEPS),
                _SideWork(wo_jobs, 2, 28, t >= V_STEPS)]

        def product(o, i):
            p = _dot(_get(a2, 7 * o + i, start, v_rows), _get(o2, 7 * o + i, (half, qd, 0), qd, _lanes(0)))
            for s in work:
                s.step(p)
            return p

        def emit(s, q, v):
            i, k = _block(s, q)
            qkv[2, 2 * k + half, _rows(_plus(start, first_row(i)), v_rows), :] = v

        _two_levels(product, emit)
        return carry

    jax.lax.fori_loop(0, V_STEPS, v_body, 0)
    middle = first_row(2) - HALO
    for m in (1, 2):
        for c in range(8):
            qkv[m, c, :HALO, :] = jnp.broadcast_to(qkv[m, c, HALO:HALO + 1, :], (HALO, LANES))
            qkv[m, c, middle:middle + HALO, :] = qkv[m, c, middle - HALO:middle, :]

    groups = qm // GROUP // nf

    def ffn_body(j, carry):
        slot = j % 2

        @pl.when(j + 1 < nf)
        def _():
            for c in f_copies(j + 1, 1 - slot):
                c.start()

        for c in f_copies(j, slot):
            c.wait()

        units, jobs = [], []
        for n in range(groups + 1):
            start = (j, groups * GROUP, n * GROUP)
            rows, swap = [_plus(start, first_row(q)) for q in range(4)], None
            if n == groups:
                g = jnp.where(j < qm // GROUP - nf * groups, j, 0)
                start, swap = (g, GROUP, nf * groups * GROUP), g % 2
                shift = swap * ((first_row(2) - first_row(0)) // GROUP)
                rows = [((g + shift if q < 2 else g - shift) // 2, 2 * GROUP, start[2] + first_row(q))
                        for q in range(4)]
            att = [[] for _ in range(4)]
            units += [_attention(qkv, rows[q], att[q]) for q in range(4)]

            def load(att, swap, p, after):
                return [[att[q][2 * k + p] if swap is None else
                         jnp.where(swap == 1, att[q ^ 2][2 * k + p], att[q][2 * k + p])
                         for k in range(4)] for q in range(4)]

            for p in range(2):
                jobs += _split_jobs(LHS, functools.partial(load, att, swap, p),
                                    lambda k, v, start=start, p=p: _put(o2, k, start, _lanes(p), v))
        for u in range(len(units) + 2):
            for stage, lag in enumerate((0, 2, 2)):
                if 0 <= u - lag < len(units):
                    units[u - lag][stage]()
        work = _SideWork(jobs, 18, 96, j >= nf)

        def w_in(s, q):
            i, k = _block(s, q)
            r, c = slice(i * qd, (i + 1) * qd), slice(k * qf, (k + 1) * qf)
            return jnp.concatenate([wg_v[slot, r, c].astype(F32), wu_v[slot, r, c].astype(F32)], axis=1)

        def w_out(s, q):
            i, k = _block(s, q)
            return jnp.concatenate([wd_v[slot, i * qf:(i + 1) * qf, _lanes(4 * p + k)].astype(F32)
                                    for p in range(2)], axis=1)

        def operand(spec, o, i, get):
            return _comb(spec[i], lambda s: _comb(spec[o], lambda q: get(s, q))).astype(BF16)

        def product(o, i):
            p = _dot(_get(a2, 7 * o + i, 0, qm), operand(RHS, o, i, w_in))
            work.step(p)
            return p

        h = _Parked(hid, j // nf)

        def gate(s, q, v):
            h[4 * s + q] = v[:, :qf] * v[:, qf:]

        _two_levels(product, gate, lambda k: _Parked(tmp[5 * k:], j // nf))
        for o in (2, 4, 5, 3, 1, 6, 0):
            for i in (3, 2, 4, 5, 1, 6, 0):
                p = _dot(operand(LHS, o, i, lambda s, q: h[4 * s + q]), operand(RHS, o, i, w_out))
                for c in range(2):
                    acc[7 * o + i, c] += p[:, _lanes(c)]
                work.step(p)
        return carry

    jax.lax.fori_loop(0, nf, ffn_body, 0)

    def out_body(t, carry):
        start, half = (t // 2, out_rows, 0), t % 2

        def product(o, i):
            p = _dot(_get(o2, 7 * o + i, start, out_rows), _get(wo2, 2 * (7 * o + i) + half, 0, qd))
            return p + acc[7 * o + i, half, _rows(start, out_rows), :]

        def emit(s, q, v):
            i, k = _block(s, q)
            at = (i, _rows(start, out_rows), _rows((half, hd, k * LANES), LANES))
            x_v[at] = (x_v[at].astype(F32) + v).astype(BF16)

        _two_levels(product, emit)
        out_copy(t).start()
        return carry

    jax.lax.fori_loop(0, OUT_STEPS, out_body, 0)
    for t in range(OUT_STEPS):
        out_copy(t).wait()


@jax.jit
def pallas_parallel_sum__sliding_local_dilated__glu_gated_bilinear__prompt_kernel(
    A_x: jax.Array,
    A_wqkv: jax.Array,
    A_wo: jax.Array,
    B_x: jax.Array,
    B_w_gate: jax.Array,
    B_w_up: jax.Array,
    B_w_down: jax.Array,
):
    del B_x
    b, s, d = A_x.shape
    assert (b, s, d, B_w_gate.shape[1]) == (1, 2048, 8 * LANES, 28 * LANES)
    qm, tf = s // 4, 4 * LANES
    any_spec = pl.BlockSpec(memory_space=pl.ANY)
    out = pl.pallas_call(
        _kernel,
        in_specs=[any_spec] * 6,
        out_specs=any_spec,
        out_shape=jax.ShapeDtypeStruct((4, qm, d), A_x.dtype),
        scratch_shapes=[
            pltpu.VMEM((4, qm, d), BF16),
            pltpu.VMEM((2, d, tf), BF16),
            pltpu.VMEM((2, d, tf), BF16),
            pltpu.VMEM((2, tf, d), BF16),
            pltpu.VMEM((49, qm // 2, d // 4), U32),
            pltpu.VMEM((98, d // 8, LANES), U32),
            pltpu.VMEM((49, 2, qm, LANES), F32),
            pltpu.VMEM((3, 8, s + 2 * HALO + 8, LANES), F32),
            pltpu.VMEM((2, 2, d // 2, d), BF16),
            [pltpu.VMEM((2, qm // 2, d // 2), U32)] * 7,
            pltpu.VMEM((49, qm // 2, d // 4), U32),
            [pltpu.VMEM((qm, tf // 2), F32)] * 25,
            [pltpu.VMEM((qm, tf // 4), F32)] * 16,
            pltpu.SemaphoreType.DMA((2, FIRST_STEPS)),
            pltpu.SemaphoreType.DMA((2 + Q_STEPS,)),
            pltpu.SemaphoreType.DMA((3, 2)),
            pltpu.SemaphoreType.DMA((OUT_STEPS,)),
        ],
        compiler_params=pltpu.CompilerParams(
            vmem_limit_bytes=127 * 2 ** 20,
            disable_bounds_checks=True,
            flags={"XLA_TPU_EVENLY_DISTRIBUTE_CRITICAL_NODES": True},
        ),
    )(A_x.reshape(4, qm, d), A_wqkv.reshape(2, d // 2, 3 * d), A_wo.reshape(2, d // 2, d),
      B_w_gate, B_w_up, B_w_down)
    return out.reshape(b, s, d)
```
